```python
import jax
import jax.numpy as jnp

def _softmax(x, axis=-1):
    return jax.nn.softmax(x, axis=axis)
def _gelu(x):
    return jax.nn.gelu(x, approximate=True)
def _silu(x):
    return jax.nn.silu(x)
def _sigmoid(x):
    return jax.nn.sigmoid(x)
def _layernorm(x, axis=-1, eps=1e-5):
    m = jnp.mean(x, axis=axis, keepdims=True)
    v = jnp.var(x, axis=axis, keepdims=True)
    return (x - m) / jnp.sqrt(v + eps)
def _scatter_add(tgt, idx, src, axis=0):
    return tgt.at[idx].add(src)
def _segment_sum(src, seg, n):
    return jax.ops.segment_sum(src, seg, n)
class _Rng:
    def __init__(self, key):
        self._k = key
    def _next(self):
        self._k, sub = jax.random.split(self._k)
        return sub
    def normal(self, shape):
        return jax.random.normal(self._next(), shape, dtype=jnp.bfloat16)
    def randint(self, lo, hi, shape):
        return jax.random.randint(self._next(), shape, lo, hi, dtype=jnp.int32)
    def uniform(self, shape, lo=0.0, hi=1.0):
        return jax.random.uniform(self._next(), shape, jnp.bfloat16, lo, hi)
    def permutation(self, n):
        return jax.random.permutation(self._next(), n)


kernel_name = 'interleave_layers__ssm_conv_h3__mixer_s_mlp__prompt'

def setup_inputs():
    _rng = _Rng(jax.random.key(int.from_bytes(__import__("os").urandom(4), "little")))
    _w = (lambda a: (lambda t: t.astype(jnp.bfloat16) if jnp.issubdtype(t.dtype, jnp.floating) else t)(jnp.asarray(a)))
    def _A_setup():
        B, S, D = 1, 2048, 1024
        ks = 4
        return {
            "q": _w((lambda *s: _rng.normal(s) * 0.05)(B, S, D)),
            "k": _w((lambda *s: _rng.normal(s) * 0.05)(B, S, D)),
            "v": _w((lambda *s: _rng.normal(s) * 0.05)(B, S, D)),
            "shift_k": _w((lambda *s: _rng.normal(s) * 0.05)(D, ks) * 0.5),
            "ssm_k": _w((lambda *s: _rng.normal(s) * 0.05)(D, S) * (1.0 / S ** 0.5)),
            "ssm_D": _w((lambda *s: _rng.normal(s) * 0.05)(D)),
        }
    _A_in = _A_setup()

    def _B_setup():
        B, S, D, F = 1, 2048, 1024, 3584
        return {
            "x":  _w((lambda *s: _rng.normal(s) * 0.05)(B, S, D)),
            "w1": _w((lambda *s: _rng.normal(s) * 0.05)(D, D) * (D ** -0.5)),
            "w2": _w((lambda *s: _rng.normal(s) * 0.05)(D, D) * (D ** -0.5)),
            "w3": _w((lambda *s: _rng.normal(s) * 0.05)(D, F) * (D ** -0.5)),
            "w4": _w((lambda *s: _rng.normal(s) * 0.05)(F, D) * (F ** -0.5)),
        }
    _B_in = _B_setup()

    return {
        "A_q": _A_in["q"],
        "A_k": _A_in["k"],
        "A_v": _A_in["v"],
        "A_shift_k": _A_in["shift_k"],
        "A_ssm_k": _A_in["ssm_k"],
        "A_ssm_D": _A_in["ssm_D"],
        "B_x": _B_in["x"],
        "B_w1": _B_in["w1"],
        "B_w2": _B_in["w2"],
        "B_w3": _B_in["w3"],
        "B_w4": _B_in["w4"],
    }

def reference(A_q, A_k, A_v, A_shift_k, A_ssm_k, A_ssm_D, B_x, B_w1, B_w2, B_w3, B_w4):
    def _A_ref(q, k, v, shift_k, ssm_k, ssm_D):
        B, S, D = q.shape
        ks = shift_k.shape[-1]
        k_pad = jnp.pad(k, ((0, 0), (ks - 1, 0), (0, 0)))
        k_shift = jnp.zeros_like(k)
        for t in range(ks):
            k_shift = k_shift + k_pad[:, t:t + S, :] * shift_k[:, ks - 1 - t][None, None, :]
        kv = k_shift * v
        L = 2 * S
        kv_pad = jnp.pad(kv, ((0, 0), (0, S), (0, 0)))
        kf_pad = jnp.pad(ssm_k, ((0, 0), (0, S)))
        kv_f = (lambda x, axes=(-2,-1): jnp.fft.rfft2(x.astype(jnp.float32), axes=axes))(kv_pad[:, None, :, :], axes=(1, 2))
        kf_f = (lambda x, axes=(-2,-1): jnp.fft.rfft2(x.astype(jnp.float32), axes=axes))(kf_pad[:, None, :], axes=(1, 2))
        kf_f = (lambda x, *d: x.transpose(*d))(kf_f, 1, 2, 0)
        y_f = kv_f * kf_f[None, :, :, :]
        y = (lambda x, s, axes=(-2,-1): jnp.fft.irfft2(x, s=s, axes=axes).astype(jnp.bfloat16))(y_f, (1, L), axes=(1, 2))[:, 0, :S, :]
        y = y + kv * ssm_D[None, None, :]
        return q * y

    def _B_ref(x, w1, w2, w3, w4):
        B, S, D = x.shape
        h = _gelu(_layernorm(x, axis=-1) @ w1)
        c = D // 4
        g0 = jnp.pad(h[:, :, 0*c:1*c], ((0, 0), (1, 0), (0, 0)))[:, :S, :]
        g1 = jnp.pad(h[:, :, 1*c:2*c], ((0, 0), (0, 1), (0, 0)))[:, 1:, :]
        g2 = jnp.pad(h[:, :, 2*c:3*c], ((0, 0), (2, 0), (0, 0)))[:, :S, :]
        g3 = jnp.pad(h[:, :, 3*c:   ], ((0, 0), (0, 2), (0, 0)))[:, 2:, :]
        hs = jnp.concatenate([g0, g1, g2, g3], axis=-1) @ w2
        x1 = x + hs
        h2 = _gelu(_layernorm(x1, axis=-1) @ w3) @ w4
        return x1 + h2

    x = A_q
    x = x + _A_ref(_layernorm(x, axis=-1), A_k, A_v, A_shift_k, A_ssm_k, A_ssm_D)
    x = x + _B_ref(_layernorm(x, axis=-1), B_w1, B_w2, B_w3, B_w4)
    x = x + _A_ref(_layernorm(x, axis=-1), A_k, A_v, A_shift_k, A_ssm_k, A_ssm_D)
    x = x + _B_ref(_layernorm(x, axis=-1), B_w1, B_w2, B_w3, B_w4)
    return x
```

```python
import numpy as np
import jax
import jax.numpy as jnp
from jax import lax
import jax.experimental.pallas as pl
import jax.experimental.pallas.tpu as pltpu

S, D, F = 2048, 1024, 3584
KS = 4
C = 128
NC = S // C
W = 256
NW = D // W
BM = 256
NB = S // BM
HALO = 8
EPS = 1e-5
BF = jnp.bfloat16
F32 = jnp.float32


def _dft_mats():
    f = np.concatenate([np.arange(0, C, 2), np.arange(1, C, 2)])
    th = 2.0 * np.pi * (f[:, None] + 0.5) * np.arange(C)[None, :] / (2 * C)
    fwd = np.concatenate([np.cos(th), -np.sin(th)], 0)
    inv = np.concatenate([np.cos(th).T, -np.sin(th).T], 1) / C
    return np.asarray(fwd, dtype=BF), np.asarray(inv, dtype=BF)


def _ln(x):
    m = jnp.mean(x, axis=-1, keepdims=True)
    d = x - m
    v = jnp.mean(d * d, axis=-1, keepdims=True)
    return d * lax.rsqrt(v + EPS)


def _gelu(x):
    c0 = 0.7978845608028654
    u = x * (x * x * (c0 * 0.044715) + c0)
    hx = 0.5 * x
    return hx * jnp.tanh(u) + hx


def _dot(a, b):
    return jnp.dot(a, b, preferred_element_type=F32)


def _kernel(q_hbm, k_hbm, v_hbm, sk_ref, kk_hbm, d_ref, w1_hbm, w2_hbm, w3_hbm, w4_hbm,
            fwd_ref, inv_ref, o_hbm,
            q_v, k_v, v_v, kk_v, w1_v, w2_v, w3_v, w4_v,
            kpad, xs, ks, y_v, x_v, xn_v, h_v, o_v, sem_c, sem_w, sem_o):
    def conv_copies(c):
        return (
            pltpu.make_async_copy(k_hbm.at[:, pl.ds(c * W, W)], k_v.at[c], sem_c.at[0, c]),
            pltpu.make_async_copy(v_hbm.at[:, pl.ds(c * W, W)], v_v.at[c], sem_c.at[1, c]),
            pltpu.make_async_copy(kk_hbm.at[pl.ds(c * W, W), :], kk_v.at[c], sem_c.at[2, c]),
        )

    w_copies = [
        pltpu.make_async_copy(q_hbm, q_v, sem_w.at[0]),
        pltpu.make_async_copy(w1_hbm, w1_v, sem_w.at[1]),
        pltpu.make_async_copy(w2_hbm, w2_v, sem_w.at[2]),
        pltpu.make_async_copy(w3_hbm, w3_v, sem_w.at[3]),
        pltpu.make_async_copy(w4_hbm, w4_v, sem_w.at[4]),
    ]
    for c in range(NW):
        for cp in conv_copies(c):
            cp.start()
    for cp in w_copies:
        cp.start()

    kpad[0:HALO, :] = jnp.zeros((HALO, W), F32)
    h_v[0:HALO, :] = jnp.zeros((HALO, D), F32)
    h_v[HALO + S:, :] = jnp.zeros((HALO, D), F32)

    def conv_block(c, carry):
        for cp in conv_copies(c):
            cp.wait()
        sk = sk_ref[c]
        fwd = fwd_ref[...]
        for j in range(NC):
            kpad[HALO + j * C:HALO + (j + 1) * C, :] = k_v[c, j * C:(j + 1) * C, :].astype(F32)
        for j in range(NC):
            acc = None
            for d in range(KS):
                t = kpad[HALO + j * C - d:HALO + (j + 1) * C - d, :] * sk[d:d + 1, :]
                acc = t if acc is None else acc + t
            kv = (acc * v_v[c, j * C:(j + 1) * C, :].astype(F32)).astype(BF)
            v_v[c, j * C:(j + 1) * C, :] = kv
            xs[j] = _dot(fwd, kv)
            ks[j] = lax.dot_general(fwd, kk_v[c, :, j * C:(j + 1) * C],
                                    (((1,), (1,)), ((), ())), preferred_element_type=F32)
        H = C // 2
        for m in range(NC - 1, 0, -1):
            ks[m, 0:H] = ks[m, 0:H] - ks[m - 1, C:C + H]
            ks[m, H:C] = ks[m, H:C] + ks[m - 1, C + H:2 * C]
            ks[m, C:C + H] = ks[m, C:C + H] + ks[m - 1, 0:H]
            ks[m, C + H:2 * C] = ks[m, C + H:2 * C] - ks[m - 1, H:C]

        def ftile(ft, carry):
            r = pl.ds(pl.multiple_of(ft * 8, 8), 8)
            i_ = pl.ds(pl.multiple_of(C + ft * 8, 8), 8)
            for j in range(NC - 1, -1, -1):
                zr = zi = None
                for i in range(j + 1):
                    xr, xi = xs[i, r, :], xs[i, i_, :]
                    kr, ki = ks[j - i, r, :], ks[j - i, i_, :]
                    tr = xr * kr - xi * ki
                    ti = xr * ki + xi * kr
                    zr = tr if zr is None else zr + tr
                    zi = ti if zi is None else zi + ti
                xs[j, r, :] = zr
                xs[j, i_, :] = zi
            return carry

        lax.fori_loop(0, C // 8, ftile, 0)
        inv = inv_ref[...]
        off = pl.multiple_of(c * W, W)
        for j in range(NC):
            y = _dot(inv, xs[j].astype(BF))
            y = y + v_v[c, j * C:(j + 1) * C, :].astype(F32) * sk[4:5, :]
            y_v[j * C:(j + 1) * C, pl.ds(off, W)] = y.astype(BF)
        return carry

    lax.fori_loop(0, NW, conv_block, 0)

    for cp in w_copies:
        cp.wait()

    def init_x(b, carry):
        rows = pl.ds(pl.multiple_of(b * BM, BM), BM)
        x_v[rows, :] = q_v[rows, :].astype(F32)
        return carry

    lax.fori_loop(0, NB, init_x, 0)

    def out_copy(b):
        rows = pl.ds(pl.multiple_of(b * BM, BM), BM)
        return pltpu.make_async_copy(o_v.at[rows, :], o_hbm.at[rows, :], sem_o.at[b])

    def layer(l, carry):
        def phase_a(b, carry):
            r0 = pl.multiple_of(b * BM, BM)
            rows = pl.ds(r0, BM)
            x = x_v[rows, :]
            x = x + _ln(x) * y_v[rows, :].astype(F32)
            x_v[rows, :] = x
            xn = _ln(x)
            xn_v[rows, :] = xn
            h = _gelu(_dot(_ln(xn).astype(BF), w1_v[...]))
            h_v[pl.ds(pl.multiple_of(r0 + HALO, 8), BM), :] = h
            return carry

        lax.fori_loop(0, NB, phase_a, 0)

        def phase_b(b, carry):
            r0 = pl.multiple_of(b * BM, BM)
            rows = pl.ds(r0, BM)
            Q = D // 4
            gs = []
            for g, sh in enumerate((-1, 1, -2, 2)):
                win = h_v[pl.ds(r0, BM + 2 * HALO), g * Q:(g + 1) * Q]
                gs.append(win[HALO + sh:HALO + sh + BM, :].astype(BF))
            x1 = xn_v[rows, :] + _dot(jnp.concatenate(gs, axis=1), w2_v[...])
            h2 = _gelu(_dot(_ln(x1).astype(BF), w3_v[...])).astype(BF)
            x = x_v[rows, :] + x1 + _dot(h2, w4_v[...])
            x_v[rows, :] = x
            o_v[rows, :] = x.astype(BF)

            @pl.when(l == 1)
            def _():
                out_copy(b).start()
            return carry

        lax.fori_loop(0, NB, phase_b, 0)
        return carry

    lax.fori_loop(0, 2, layer, 0)
    for b in range(NB):
        out_copy(b).wait()


@jax.jit
def pallas_interleave_layers__ssm_conv_h3__mixer_s_mlp__prompt_kernel(
    A_q, A_k, A_v, A_shift_k, A_ssm_k, A_ssm_D, B_x, B_w1, B_w2, B_w3, B_w4,
):
    fwd, inv = _dft_mats()
    sk = jnp.concatenate([A_shift_k.T, A_ssm_D[None, :], jnp.zeros((3, D), BF)], 0)
    sk = sk.astype(F32).reshape(8, NW, W).transpose(1, 0, 2)
    hbm = pl.BlockSpec(memory_space=pl.ANY)
    vm = pl.BlockSpec(memory_space=pltpu.VMEM)
    out = pl.pallas_call(
        _kernel,
        in_specs=[hbm, hbm, hbm, vm, hbm, vm, hbm, hbm, hbm, hbm, vm, vm],
        out_specs=hbm,
        out_shape=jax.ShapeDtypeStruct((S, D), BF),
        scratch_shapes=[
            pltpu.VMEM((S, D), BF), pltpu.VMEM((NW, S, W), BF), pltpu.VMEM((NW, S, W), BF),
            pltpu.VMEM((NW, W, S), BF),
            pltpu.VMEM((D, D), BF), pltpu.VMEM((D, D), BF),
            pltpu.VMEM((D, F), BF), pltpu.VMEM((F, D), BF),
            pltpu.VMEM((S + HALO, W), F32),
            pltpu.VMEM((NC, 2 * C, W), F32), pltpu.VMEM((NC, 2 * C, W), F32),
            pltpu.VMEM((S, D), BF), pltpu.VMEM((S, D), F32), pltpu.VMEM((S, D), F32),
            pltpu.VMEM((S + 2 * HALO, D), F32), pltpu.VMEM((S, D), BF),
            pltpu.SemaphoreType.DMA((3, NW)), pltpu.SemaphoreType.DMA((5,)),
            pltpu.SemaphoreType.DMA((NB,)),
        ],
        compiler_params=pltpu.CompilerParams(vmem_limit_bytes=120 * 1024 * 1024),
    )(A_q.reshape(S, D), A_k.reshape(S, D), A_v.reshape(S, D), sk, A_ssm_k,
      A_ssm_D.reshape(1, D), B_w1, B_w2, B_w3, B_w4, fwd, inv)
    return out.reshape(1, S, D)
```

```python
import functools
import numpy as np
import jax
import jax.numpy as jnp
from jax import lax
import jax.experimental.pallas as pl
import jax.experimental.pallas.tpu as pltpu

S, D, F = 2048, 1024, 3584
KS = 4
JB = 4
C = 128
NC = S // C
W = 256
NW = D // W
BM = 256
NB = S // BM
HALO = 8
EPS = 1e-5
BF = jnp.bfloat16
F32 = jnp.float32


def _dft_mats():
    f = np.concatenate([np.arange(0, C, 2), np.arange(1, C, 2)])
    th = 2.0 * np.pi * (f[:, None] + 0.5) * np.arange(C)[None, :] / (2 * C)
    fwd = np.concatenate([np.cos(th), -np.sin(th)], 0)
    inv = np.concatenate([np.cos(th).T, -np.sin(th).T], 1) / C
    return np.asarray(fwd, dtype=BF), np.asarray(inv, dtype=BF)


def _ln(x):
    m = jnp.mean(x, axis=-1, keepdims=True)
    d = x - m
    v = jnp.mean(d * d, axis=-1, keepdims=True)
    return d * lax.rsqrt(v + EPS)


def _gelu(x):
    c0 = 0.7978845608028654
    u = x * (x * x * (c0 * 0.044715) + c0)
    hx = 0.5 * x
    return hx * jnp.tanh(u) + hx


def _dot(a, b):
    return jnp.dot(a, b, preferred_element_type=F32)


def _kernel(q_hbm, k_hbm, v_hbm, sk_ref, kk_hbm, d_ref, w1_hbm, w2_hbm, w3_hbm, w4_hbm,
            fwd_ref, inv_ref, o_hbm,
            q_v, k_v, v_v, kk_v, w1_v, w2_v, w3_v, w4_v,
            kpad, xs, ks, y_v, x_v, xn_v, h_v, o_v, la, lb, gb, sem_c, sem_w, sem_o):
    def conv_copies(c):
        return (
            pltpu.make_async_copy(k_hbm.at[:, pl.ds(c * W, W)], k_v.at[c], sem_c.at[0, c]),
            pltpu.make_async_copy(v_hbm.at[:, pl.ds(c * W, W)], v_v.at[c], sem_c.at[1, c]),
            pltpu.make_async_copy(kk_hbm.at[pl.ds(c * W, W), :], kk_v.at[c], sem_c.at[2, c]),
        )

    w_copies = [
        pltpu.make_async_copy(q_hbm, q_v, sem_w.at[0]),
        pltpu.make_async_copy(w1_hbm, w1_v, sem_w.at[1]),
        pltpu.make_async_copy(w2_hbm, w2_v, sem_w.at[2]),
        pltpu.make_async_copy(w3_hbm, w3_v, sem_w.at[3]),
        pltpu.make_async_copy(w4_hbm, w4_v, sem_w.at[4]),
    ]
    for c in range(1):
        for cp in conv_copies(c):
            cp.start()

    kpad[0:HALO, :] = jnp.zeros((HALO, W), F32)
    h_v[0:HALO, :] = jnp.zeros((HALO, D), F32)
    h_v[HALO + S:, :] = jnp.zeros((HALO, D), F32)

    def conv_block(c, carry):
        for cp in conv_copies(c):
            cp.wait()

        @pl.when(c + 1 < NW)
        def _():
            for cp in conv_copies(jnp.minimum(c + 1, NW - 1)):
                cp.start()

        @pl.when(c == NW - 1)
        def _():
            w_copies[0].start()
            w_copies[1].start()
            w_copies[2].start()

        off = pl.multiple_of(c * W, W)
        sk = sk_ref[:, pl.ds(off, W)].astype(F32)
        skip = d_ref[:, pl.ds(off, W)].astype(F32)
        fwd = fwd_ref[...]
        for j in range(NC):
            kpad[HALO + j * C:HALO + (j + 1) * C, :] = k_v[c, j * C:(j + 1) * C, :].astype(F32)
        for j in range(NC):
            acc = None
            for d in range(KS):
                t = kpad[HALO + j * C - d:HALO + (j + 1) * C - d, :] * sk[d:d + 1, :]
                acc = t if acc is None else acc + t
            kv = (acc * v_v[c, j * C:(j + 1) * C, :].astype(F32)).astype(BF)
            v_v[c, j * C:(j + 1) * C, :] = kv
            xf = _dot(fwd, kv)
            kf = lax.dot_general(fwd, kk_v[c, :, j * C:(j + 1) * C],
                                 (((1,), (1,)), ((), ())), preferred_element_type=F32)
            xs[j, 0:2 * C] = xf
            xs[j, 2 * C:] = xf[:C] + xf[C:]
            ks[j, 0:C] = kf[C:] - kf[:C]
            ks[j, C:2 * C] = kf[C:] + kf[:C]
            ks[j, 2 * C:] = kf[:C]

        def ftile(ft, sgn):
            rs = [pl.ds(pl.multiple_of(t * C + ft * 8, 8), 8) for t in range(3)]
            for lt in range(W // 128):
                ln = slice(lt * 128, (lt + 1) * 128)
                prev = None
                for j0 in range(NC - JB, -1, -JB):
                    acc = [[None] * 3 for _ in range(JB)]
                    for i in range(j0 + JB):
                        for t in range(3):
                            xv = xs[i, rs[t], ln]
                            for u in range(JB):
                                if j0 + u >= i:
                                    m = xv * ks[j0 + u - i, rs[t], ln]
                                    acc[u][t] = m if acc[u][t] is None else acc[u][t] + m
                    for u in range(JB - 1, -1, -1):
                        yr, yi = acc[u][2] - acc[u][1], acc[u][2] + acc[u][0]
                        if prev is not None:
                            pr, pi = prev
                            xs[j0 + u + 1, rs[0], ln] = pr - yi if sgn > 0 else pr + yi
                            xs[j0 + u + 1, rs[1], ln] = pi + yr if sgn > 0 else pi - yr
                        prev = (yr, yi)
                xs[0, rs[0], ln] = prev[0]
                xs[0, rs[1], ln] = prev[1]
            return sgn

        lax.fori_loop(0, C // 16, lambda t, cr: (ftile(t, 1), cr)[1], 0)
        lax.fori_loop(C // 16, C // 8, lambda t, cr: (ftile(t, -1), cr)[1], 0)
        inv = inv_ref[...]
        for j in range(NC):
            y = _dot(inv, xs[j, 0:2 * C].astype(BF))
            y = y + v_v[c, j * C:(j + 1) * C, :].astype(F32) * skip
            y_v[j * C:(j + 1) * C, pl.ds(off, W)] = y.astype(BF)
        return carry

    lax.fori_loop(0, NW, conv_block, 0)

    def blk(v, r=0, n=BM):
        return pl.ds(pl.multiple_of((v % NB) * BM + r, 8), n)

    RP = 64
    NP = BM // RP

    def prep(v, src, p):
        rows = blk(v, p * RP, RP)
        x = src[rows, :].astype(F32)
        x = x + _ln(x) * y_v[rows, :].astype(F32)
        x_v[rows, :] = x
        xn = _ln(x)
        xn_v[rows, :] = xn
        la[v % 2, p * RP:(p + 1) * RP, :] = _ln(xn).astype(BF)

    def shift(v, p):
        Q = D // 4
        for g, sh in enumerate((-1, 1, -2, 2)):
            win = h_v[blk(v, p * RP, RP + 2 * HALO), g * Q:(g + 1) * Q]
            gb[v % 2, p * RP:(p + 1) * RP, g * Q:(g + 1) * Q] = (
                win[HALO + sh:HALO + sh + RP, :].astype(BF))

    def ln1(v, p):
        lb[v % 2, p * RP:(p + 1) * RP, :] = _ln(xn_v[blk(v, p * RP, RP), :]).astype(BF)

    NCH = 256

    def mix_a(v, fill=()):
        for n in range(D // NCH):
            cols = slice(n * NCH, (n + 1) * NCH)
            h_v[blk(v, HALO), cols] = _gelu(_dot(la[v % 2], w1_v[:, cols]))
            for f in fill[n::D // NCH]:
                f()

    def mix_b(v, fill=()):
        for n in range(D // NCH):
            cols = slice(n * NCH, (n + 1) * NCH)
            xn_v[blk(v), cols] = xn_v[blk(v), cols] + _dot(gb[v % 2], w2_v[:, cols])
            for f in fill[n::D // NCH]:
                f()

    def mlp(v, fill=()):
        rows = blk(v)
        h2 = _gelu(_dot(lb[v % 2], w3_v[...])).astype(BF)
        NO = 128
        for n in range(D // NO):
            cols = slice(n * NO, (n + 1) * NO)
            x = x_v[rows, cols] + xn_v[rows, cols] + _dot(h2, w4_v[:, cols])
            x_v[rows, cols] = x
            o_v[rows, cols] = x.astype(BF)
            for f in (fill[n // 2::D // NO // 2] if n % 2 == 0 else ()):
                f()

    def pieces(fn, *args):
        return [functools.partial(fn, *args, p) for p in range(NP)]

    def run(fs):
        for f in fs:
            f()

    def out_copy(v):
        return pltpu.make_async_copy(o_v.at[blk(v), :], o_hbm.at[blk(v), :], sem_o.at[v % NB])

    SK = 6
    q_cp, w1_cp, w2_cp, w3_cp, w4_cp = w_copies
    q_cp.wait()
    w3_cp.start()
    x_v[(NB - 1) * BM:, :] = q_v[(NB - 1) * BM:, :].astype(F32)
    run(pieces(prep, 0, q_v))
    w1_cp.wait()
    w4_cp.start()

    def pro(v, carry):
        mix_a(v, pieces(prep, v + 1, q_v))
        return carry

    lax.fori_loop(0, SK, pro, 0)
    w2_cp.wait()
    run(pieces(shift, 0))
    mix_b(0, pieces(shift, 1))
    mix_b(1, pieces(shift, 2) + pieces(ln1, 0))
    w3_cp.wait()
    w4_cp.wait()

    def main(i, carry):
        mix_b(i + 2, pieces(shift, i + 3))
        mix_a(i + SK, pieces(ln1, i + 1))
        mlp(i, pieces(prep, i + SK + 1, x_v))

        @pl.when(i >= NB)
        def _():
            out_copy(i).start()
        return carry

    lax.fori_loop(0, 2 * NB - SK, main, 0)

    def tail(i, carry):
        mix_b(i + 2, pieces(shift, i + 3))
        mlp(i, pieces(ln1, i + 1))
        out_copy(i).start()
        return carry

    lax.fori_loop(2 * NB - SK, 2 * NB - 2, tail, 0)

    def last(i, carry):
        mlp(i, pieces(ln1, i + 1))
        out_copy(i).start()
        return carry

    lax.fori_loop(2 * NB - 2, 2 * NB, last, 0)
    for b in range(NB):
        out_copy(b).wait()


@jax.jit
def pallas_interleave_layers__ssm_conv_h3__mixer_s_mlp__prompt_kernel(
    A_q, A_k, A_v, A_shift_k, A_ssm_k, A_ssm_D, B_x, B_w1, B_w2, B_w3, B_w4,
):
    fwd, inv = _dft_mats()
    hbm = pl.BlockSpec(memory_space=pl.ANY)
    vm = pl.BlockSpec(memory_space=pltpu.VMEM)
    out = pl.pallas_call(
        _kernel,
        in_specs=[hbm, hbm, hbm, vm, hbm, vm, hbm, hbm, hbm, hbm, vm, vm],
        out_specs=hbm,
        out_shape=jax.ShapeDtypeStruct((S, D), BF),
        scratch_shapes=[
            pltpu.VMEM((S, D), BF), pltpu.VMEM((NW, S, W), BF), pltpu.VMEM((NW, S, W), BF),
            pltpu.VMEM((NW, W, S), BF),
            pltpu.VMEM((D, D), BF), pltpu.VMEM((D, D), BF),
            pltpu.VMEM((D, F), BF), pltpu.VMEM((F, D), BF),
            pltpu.VMEM((S + HALO, W), F32),
            pltpu.VMEM((NC, 3 * C, W), F32), pltpu.VMEM((NC, 3 * C, W), F32),
            pltpu.VMEM((S, D), BF), pltpu.VMEM((S, D), F32), pltpu.VMEM((S, D), F32),
            pltpu.VMEM((S + 2 * HALO, D), F32), pltpu.VMEM((S, D), BF),
            pltpu.VMEM((2, BM, D), BF), pltpu.VMEM((2, BM, D), BF), pltpu.VMEM((2, BM, D), BF),
            pltpu.SemaphoreType.DMA((3, NW)), pltpu.SemaphoreType.DMA((5,)),
            pltpu.SemaphoreType.DMA((NB,)),
        ],
        compiler_params=pltpu.CompilerParams(vmem_limit_bytes=120 * 1024 * 1024),
    )(A_q.reshape(S, D), A_k.reshape(S, D), A_v.reshape(S, D), A_shift_k.T, A_ssm_k,
      A_ssm_D.reshape(1, D), B_w1, B_w2, B_w3, B_w4, fwd, inv)
    return out.reshape(1, S, D)
```

```python
import functools
import numpy as np
import jax
import jax.numpy as jnp
from jax import lax
import jax.experimental.pallas as pl
import jax.experimental.pallas.tpu as pltpu

S, D, F = 2048, 1024, 3584
KS = 4
JB = 4
C = 128
NC = S // C
KH = 16
W = 128
NW = D // W
BM = 256
NB = S // BM
HALO = 8
EPS = 1e-5
BF = jnp.bfloat16
F32 = jnp.float32


def _dft_mats():
    f = np.concatenate([np.arange(0, C, 2), np.arange(1, C, 2)])
    th = 2.0 * np.pi * (f[:, None] + 0.5) * np.arange(C)[None, :] / (2 * C)
    fwd = np.concatenate([np.cos(th), -np.sin(th)], 0)
    inv = np.concatenate([np.cos(th).T, -np.sin(th).T], 1) / C
    return np.asarray(fwd, dtype=BF), np.asarray(inv, dtype=BF)


def _ln(x):
    m = jnp.mean(x, axis=-1, keepdims=True)
    d = x - m
    v = jnp.mean(d * d, axis=-1, keepdims=True)
    return d * lax.rsqrt(v + EPS)


def _gelu(x):
    c0 = 0.7978845608028654
    u = x * (x * x * (c0 * 0.044715) + c0)
    hx = 0.5 * x
    return hx * jnp.tanh(u) + hx


def _dot(a, b):
    return jnp.dot(a, b, preferred_element_type=F32)


def _kernel(q_hbm, k_hbm, v_hbm, sk_ref, kk_hbm, d_ref, w1_hbm, w2_hbm, w3_hbm, w4_hbm,
            fwd_ref, inv_ref, o_hbm,
            q_v, k_v, v_v, kk_v, w1_v, w2_v, w3_v, w4_v,
            taps, xs0, xs1, ks0, ks1, zs0, zs1, kvs0, kvs1, y_v, x_v, xn_v, h_v, o_v, la, lb, gb, sem_c, sem_w, sem_o):

    xs, ks, zs, kvs = (xs0, xs1), (ks0, ks1), (zs0, zs1), (kvs0, kvs1)

    def conv_copies(c):
        cols = pl.ds(pl.multiple_of(c * W, W), W)
        return (
            pltpu.make_async_copy(k_hbm.at[:, cols], k_v.at[c, pl.ds(KH, S), :], sem_c.at[0, c]),
            pltpu.make_async_copy(v_hbm.at[:, cols], v_v.at[c], sem_c.at[1, c]),
            pltpu.make_async_copy(kk_hbm.at[cols, :], kk_v.at[c], sem_c.at[2, c]),
        )

    w_copies = [
        pltpu.make_async_copy(q_hbm, q_v, sem_w.at[0]),
        pltpu.make_async_copy(w1_hbm, w1_v, sem_w.at[1]),
        pltpu.make_async_copy(w2_hbm, w2_v, sem_w.at[2]),
        pltpu.make_async_copy(w3_hbm, w3_v, sem_w.at[3]),
        pltpu.make_async_copy(w4_hbm, w4_v, sem_w.at[4]),
    ]
    AHEAD = 3
    for c in range(1):
        for cp in conv_copies(c):
            cp.start()

    for c in range(NW):
        k_v[c, 0:KH, :] = jnp.zeros((KH, W), BF)
        taps[c, 0:KS, :] = sk_ref[c * W:(c + 1) * W, :].astype(F32).T
        taps[c, KS:KS + 1, :] = d_ref[:, c * W:(c + 1) * W].astype(F32)
    h_v[0:HALO, :] = jnp.zeros((HALO, D), F32)
    h_v[HALO + S:, :] = jnp.zeros((HALO, D), F32)

    def conv_fwd(c, j, sl):
        t0 = j * C
        tp = taps[c]
        win = k_v[c, pl.ds(t0, C + KH), :].astype(F32)
        acc = win[KH:, :] * tp[0:1, :]
        for d in range(1, KS):
            acc = acc + win[KH - d:KH - d + C, :] * tp[d:d + 1, :]
        kv = (acc * v_v[c, pl.ds(t0, C), :].astype(F32)).astype(BF)
        xf = _dot(fwd_ref[...], kv)
        kf = lax.dot_general(fwd_ref[...], kk_v[c, :, pl.ds(t0, C)],
                                       (((1,), (1,)), ((), ())), preferred_element_type=F32)

        def store():
            kvs[sl][pl.ds(t0, C), :] = kv
            xs[sl][j, 0:2 * C] = xf
            xs[sl][j, 2 * C:] = xf[:C] + xf[C:]
            ks[sl][j, 0:C] = kf[C:] - kf[:C]
            ks[sl][j, C:2 * C] = kf[C:] + kf[:C]
            ks[sl][j, 2 * C:] = kf[:C]
        return store

    def conv_mac(sl, ft, sgn):
        rs = [pl.ds(t * C + ft * 8, 8) for t in range(3)]
        prev = None
        for j0 in range(NC - JB, -1, -JB):
            acc = [[None] * 3 for _ in range(JB)]
            for i in range(j0 + JB):
                for t in range(3):
                    xv = xs[sl][i, rs[t], :]
                    for u in range(JB):
                        if j0 + u >= i:
                            m = xv * ks[sl][j0 + u - i, rs[t], :]
                            acc[u][t] = m if acc[u][t] is None else acc[u][t] + m
            for u in range(JB - 1, -1, -1):
                yr, yi = acc[u][2] - acc[u][1], acc[u][2] + acc[u][0]
                if prev is not None:
                    pr, pi = prev
                    zs[sl][j0 + u + 1, rs[0], :] = pr - yi if sgn > 0 else pr + yi
                    zs[sl][j0 + u + 1, rs[1], :] = pi + yr if sgn > 0 else pi - yr
                prev = (yr, yi)
        zs[sl][0, rs[0], :] = prev[0]
        zs[sl][0, rs[1], :] = prev[1]
        return lambda: None

    def conv_inv(c, j, sl):
        rows = pl.ds(j * C, C)
        y = _dot(inv_ref[...], zs[sl][j].astype(BF))
        y = y + kvs[sl][rows, :].astype(F32) * taps[c, KS:KS + 1, :]

        def store():
            y_v[rows, pl.ds(pl.multiple_of(c * W, W), W)] = y.astype(BF)
        return store

    for cp in conv_copies(0):
        cp.wait()
    for c in range(1, AHEAD):
        for cp in conv_copies(c):
            cp.start()

    def conv_first(t, carry):
        for st in [conv_fwd(0, t, 0), conv_fwd(0, t + NC // 2, 0)]:
            st()
        return carry

    [conv_first(t, 0) for t in range(NC // 2)]

    def conv_step(c, sl, with_fwd, with_inv=True):
        def body(t, carry):
            js = (t, t + NC // 2)
            for j, sgn in zip(js, (1, -1)):
                sts = []
                if with_fwd:
                    sts.append(conv_fwd(c + 1, j, 1 - sl))
                if with_inv:
                    sts.append(conv_inv(c - 1, j, 1 - sl))
                sts.append(conv_mac(sl, j, sgn))
                for st in sts:
                    st()
            return carry

        for t in range(NC // 2):
            body(t, 0)

    def feed(c):
        for cp in conv_copies(c + 1):
            cp.wait()

        @pl.when(c + AHEAD < NW)
        def _():
            for cp in conv_copies(jnp.minimum(c + AHEAD, NW - 1)):
                cp.start()

        for n, cp in enumerate(w_copies[:3]):
            pl.when(c == NW - AHEAD + n - 1)(cp.start)

    feed(jnp.int32(0))
    conv_step(0, 0, True, False)

    def conv_block(c, carry):
        for u in range(2):
            feed(2 * c + 1 + u)
            conv_step(2 * c + 1 + u, 1 - u, True)
        return carry

    lax.fori_loop(0, 3, conv_block, 0)
    w_copies[3].start()
    conv_step(NW - 1, (NW - 1) % 2, False)

    def conv_last(t, carry):
        for st in [conv_inv(NW - 1, t, (NW - 1) % 2), conv_inv(NW - 1, t + NC // 2, (NW - 1) % 2)]:
            st()
        return carry

    [conv_last(t, 0) for t in range(NC // 2)]

    def blk(v, r=0, n=BM):
        return pl.ds(pl.multiple_of((v % NB) * BM + r, 8), n)

    RP = 64
    NP = BM // RP

    def prep(v, src, p):
        rows = blk(v, p * RP, RP)
        x = src[rows, :].astype(F32)
        x = x + _ln(x) * y_v[rows, :].astype(F32)
        x_v[rows, :] = x
        xn = _ln(x)
        xn_v[rows, :] = xn
        la[v % 2, p * RP:(p + 1) * RP, :] = _ln(xn).astype(BF)

    def shift(v, p):
        Q = D // 4
        for g, sh in enumerate((-1, 1, -2, 2)):
            win = h_v[blk(v, p * RP, RP + 2 * HALO), g * Q:(g + 1) * Q]
            gb[v % 2, p * RP:(p + 1) * RP, g * Q:(g + 1) * Q] = (
                win[HALO + sh:HALO + sh + RP, :].astype(BF))

    def ln1(v, p):
        lb[v % 2, p * RP:(p + 1) * RP, :] = _ln(xn_v[blk(v, p * RP, RP), :]).astype(BF)

    NCH = 256

    def mix_a(v, fill=()):
        for n in range(D // NCH):
            cols = slice(n * NCH, (n + 1) * NCH)
            h_v[blk(v, HALO), cols] = _gelu(_dot(la[v % 2], w1_v[:, cols]))
            for f in fill[n::D // NCH]:
                f()

    def mix_b(v, fill=()):
        for n in range(D // NCH):
            cols = slice(n * NCH, (n + 1) * NCH)
            xn_v[blk(v), cols] = xn_v[blk(v), cols] + _dot(gb[v % 2], w2_v[:, cols])
            for f in fill[n::D // NCH]:
                f()

    def mlp(v, fill=()):
        rows = blk(v)
        h2 = _gelu(_dot(lb[v % 2], w3_v[...])).astype(BF)
        NO = 128
        for n in range(D // NO):
            cols = slice(n * NO, (n + 1) * NO)
            x = x_v[rows, cols] + xn_v[rows, cols] + _dot(h2, w4_v[:, cols])
            x_v[rows, cols] = x
            o_v[rows, cols] = x.astype(BF)
            for f in (fill[n // 2::D // NO // 2] if n % 2 == 0 else ()):
                f()

    def pieces(fn, *args):
        return [functools.partial(fn, *args, p) for p in range(NP)]

    def run(fs):
        for f in fs:
            f()

    def out_copy(v):
        return pltpu.make_async_copy(o_v.at[blk(v), :], o_hbm.at[blk(v), :], sem_o.at[v % NB])

    SK = 6
    q_cp, w1_cp, w2_cp, w3_cp, w4_cp = w_copies
    q_cp.wait()
    x_v[(NB - 1) * BM:, :] = q_v[(NB - 1) * BM:, :].astype(F32)
    run(pieces(prep, 0, q_v))
    w1_cp.wait()
    w4_cp.start()

    def pro(v, carry):
        mix_a(v, pieces(prep, v + 1, q_v))
        return carry

    lax.fori_loop(0, SK, pro, 0)
    w2_cp.wait()
    run(pieces(shift, 0))
    mix_b(0, pieces(shift, 1))
    mix_b(1, pieces(shift, 2) + pieces(ln1, 0))
    w3_cp.wait()
    w4_cp.wait()

    def main(i, carry):
        mix_b(i + 2, pieces(shift, i + 3))
        mix_a(i + SK, pieces(ln1, i + 1))
        mlp(i, pieces(prep, i + SK + 1, x_v))

        @pl.when(i >= NB)
        def _():
            out_copy(i).start()
        return carry

    lax.fori_loop(0, 2 * NB - SK, main, 0)

    def tail(i, carry):
        mix_b(i + 2, pieces(shift, i + 3))
        mlp(i, pieces(ln1, i + 1))
        out_copy(i).start()
        return carry

    lax.fori_loop(2 * NB - SK, 2 * NB - 2, tail, 0)

    def last(i, carry):
        mlp(i, pieces(ln1, i + 1))
        out_copy(i).start()
        return carry

    lax.fori_loop(2 * NB - 2, 2 * NB, last, 0)
    for b in range(NB):
        out_copy(b).wait()


@jax.jit
def pallas_interleave_layers__ssm_conv_h3__mixer_s_mlp__prompt_kernel(
    A_q, A_k, A_v, A_shift_k, A_ssm_k, A_ssm_D, B_x, B_w1, B_w2, B_w3, B_w4,
):
    fwd, inv = _dft_mats()
    hbm = pl.BlockSpec(memory_space=pl.ANY)
    vm = pl.BlockSpec(memory_space=pltpu.VMEM)
    out = pl.pallas_call(
        _kernel,
        in_specs=[hbm, hbm, hbm, vm, hbm, vm, hbm, hbm, hbm, hbm, vm, vm],
        out_specs=hbm,
        out_shape=jax.ShapeDtypeStruct((S, D), BF),
        scratch_shapes=[
            pltpu.VMEM((S, D), BF), pltpu.VMEM((NW, S + KH, W), BF), pltpu.VMEM((NW, S, W), BF),
            pltpu.VMEM((NW, W, S), BF),
            pltpu.VMEM((D, D), BF), pltpu.VMEM((D, D), BF),
            pltpu.VMEM((D, F), BF), pltpu.VMEM((F, D), BF),
            pltpu.VMEM((NW, 8, W), F32),
            *[pltpu.VMEM((NC, 3 * C, W), F32)] * 4, *[pltpu.VMEM((NC, 2 * C, W), F32)] * 2, *[pltpu.VMEM((S, W), BF)] * 2,
            pltpu.VMEM((S, D), BF), pltpu.VMEM((S, D), F32), pltpu.VMEM((S, D), F32),
            pltpu.VMEM((S + 2 * HALO, D), F32), pltpu.VMEM((S, D), BF),
            pltpu.VMEM((2, BM, D), BF), pltpu.VMEM((2, BM, D), BF), pltpu.VMEM((2, BM, D), BF),
            pltpu.SemaphoreType.DMA((3, NW)), pltpu.SemaphoreType.DMA((5,)),
            pltpu.SemaphoreType.DMA((NB,)),
        ],
        compiler_params=pltpu.CompilerParams(vmem_limit_bytes=120 * 1024 * 1024),
    )(A_q.reshape(S, D), A_k.reshape(S, D), A_v.reshape(S, D), A_shift_k, A_ssm_k,
      A_ssm_D.reshape(1, D), B_w1, B_w2, B_w3, B_w4, fwd, inv)
    return out.reshape(1, S, D)
```

```python
import functools
import numpy as np
import jax
import jax.numpy as jnp
from jax import lax
import jax.experimental.pallas as pl
import jax.experimental.pallas.tpu as pltpu

S, D, F = 2048, 1024, 3584
KS = 4
JB = 4
H = 128
C = 256
NC = S // C
KH = 16
W = 128
NW = D // W
BM = 256
NB = S // BM
HALO = 8
EPS = 1e-5
BF = jnp.bfloat16
F32 = jnp.float32


def _dft_mats():
    f = np.concatenate([np.arange(0, H, 2), np.arange(1, H, 2)])
    th = 2.0 * np.pi * (f + 0.5) / (2 * C)
    ph = th[:, None] * (2 * np.arange(H))[None, :]
    half = np.concatenate([np.cos(ph), -np.sin(ph)], 0)
    inv = np.concatenate([np.cos(ph).T, -np.sin(ph).T], 1) / C
    t = np.arange(C)[None, :]
    lo, hi = th[:, None] * t, (np.pi - th)[:, None] * t
    full = np.concatenate([np.cos(lo), -np.sin(lo), np.cos(hi), np.sin(hi)], 0)
    tw = np.stack([np.cos(th), np.sin(th)])[:, :, None] * np.ones((1, 1, W))
    return (np.asarray(half, dtype=BF), np.asarray(inv, dtype=BF), np.asarray(full, dtype=BF),
            np.asarray(tw, dtype=np.float32))


def _ln(x):
    m = jnp.mean(x, axis=-1, keepdims=True)
    d = x - m
    v = jnp.mean(d * d, axis=-1, keepdims=True)
    return d * lax.rsqrt(v + EPS)


def _gelu(x):
    c0 = 0.7978845608028654
    u = x * (x * x * (c0 * 0.044715) + c0)
    hx = 0.5 * x
    return hx * jnp.tanh(u) + hx


def _dot(a, b):
    return jnp.dot(a, b, preferred_element_type=F32)


def _kernel(q_hbm, k_hbm, v_hbm, sk_ref, kk_hbm, d_ref, w1_hbm, w2_hbm, w3_hbm, w4_hbm,
            half_hbm, inv_hbm, full_hbm, tw_hbm, o_hbm,
            half_ref, inv_ref, full_ref, tw_ref, sem_k,
            q_v, k_v, v_v, kk_v, w1_v, w2_v, w3_v, w4_v,
            taps, xs0, xs1, ks0, ks1, zs0, zs1, y_v, x_v, xn_v, h_v, o_v, la, lb, gb, sem_c, sem_w, sem_o):

    xs, ks, zs = (xs0, xs1), (ks0, ks1), (zs0, zs1)

    def conv_copies(c):
        cols = pl.ds(pl.multiple_of(c * W, W), W)
        return (
            pltpu.make_async_copy(k_hbm.at[:, cols], k_v.at[c, pl.ds(KH, S), :], sem_c.at[0, c]),
            pltpu.make_async_copy(v_hbm.at[:, cols], v_v.at[c], sem_c.at[1, c]),
            pltpu.make_async_copy(kk_hbm.at[cols, :], kk_v.at[c], sem_c.at[2, c]),
        )

    w_copies = [
        pltpu.make_async_copy(q_hbm, q_v, sem_w.at[0]),
        pltpu.make_async_copy(w1_hbm, w1_v, sem_w.at[1]),
        pltpu.make_async_copy(w2_hbm, w2_v, sem_w.at[2]),
        pltpu.make_async_copy(w3_hbm, w3_v, sem_w.at[3]),
        pltpu.make_async_copy(w4_hbm, w4_v, sem_w.at[4]),
    ]
    k_copies = [pltpu.make_async_copy(a, b, sem_k.at[n]) for n, (a, b) in enumerate(
        ((half_hbm, half_ref), (inv_hbm, inv_ref), (full_hbm, full_ref), (tw_hbm, tw_ref)))]
    for cp in k_copies:
        cp.start()
    AHEAD = 3
    for c in range(1):
        for cp in conv_copies(c):
            cp.start()

    for c in range(NW):
        k_v[c, 0:KH, :] = jnp.zeros((KH, W), BF)
        taps[c, 0:KS, :] = sk_ref[c * W:(c + 1) * W, :].astype(F32).T
        taps[c, KS:KS + 1, :] = d_ref[:, c * W:(c + 1) * W].astype(F32)
    h_v[0:HALO, :] = jnp.zeros((HALO, D), F32)
    h_v[HALO + S:, :] = jnp.zeros((HALO, D), F32)

    def even_odd(x):
        u = pltpu.bitcast(x, jnp.uint32)
        return (pltpu.bitcast(u << 16, F32), pltpu.bitcast(u & jnp.uint32(0xFFFF0000), F32))

    def conv_fwd(c, j, sl):
        tp = taps[c]
        t = [tp[d:d + 1, :] for d in range(KS)]
        ke, ko = even_odd(k_v[c, pl.ds(j * C, C + KH), :])
        ve, vo = even_odd(v_v[c, pl.ds(j * C, C), :])
        P = KH // 2
        ke0, ke1 = ke[P:], ke[P - 1:P - 1 + H]
        ko0, ko1, ko2 = ko[P:], ko[P - 1:P - 1 + H], ko[P - 2:P - 2 + H]
        kve = (ke0 * t[0] + ko1 * t[1] + ke1 * t[2] + ko2 * t[3]) * ve
        kvo = (ko0 * t[0] + ke0 * t[1] + ko1 * t[2] + ke1 * t[3]) * vo
        ef = _dot(half_ref[...], kve.astype(BF))
        of = _dot(half_ref[...], kvo.astype(BF))
        kf = lax.dot_general(full_ref[...], kk_v[c, :, pl.ds(j * C, C)],
                             (((1,), (1,)), ((), ())), preferred_element_type=F32)

        def store():
            wc, ws = tw_ref[0], tw_ref[1]
            pr = of[:H] * wc + of[H:] * ws
            pi = of[H:] * wc - of[:H] * ws
            for m, (xr, xi) in enumerate(((ef[:H] + pr, ef[H:] + pi), (ef[:H] - pr, ef[H:] - pi))):
                kr, ki = kf[2 * m * H:(2 * m + 1) * H], kf[(2 * m + 1) * H:(2 * m + 2) * H]
                if j == 0:
                    kr = kr + tp[KS:KS + 1, :]
                for n, (xv, kv) in enumerate(((xr, ki - kr), (xi, ki + kr), (xr + xi, kr))):
                    xs[sl][j, pl.ds((3 * m + n) * H, H), :] = xv
                    ks[sl][j, pl.ds((3 * m + n) * H, H), :] = kv
        return store

    def conv_mac(sl, ft, sgn):
        def mac(m, j0):
            acc = [[None] * 3 for _ in range(JB)]
            for i in range(j0 + JB):
                for n in range(3):
                    r = pl.ds((3 * m + n) * H + ft * 8, 8)
                    xv = xs[sl][i, r, :]
                    for u in range(JB):
                        if j0 + u >= i:
                            p = xv * ks[sl][j0 + u - i, r, :]
                            acc[u][n] = p if acc[u][n] is None else acc[u][n] + p
            return [(a[2] - a[1], a[2] + a[0]) for a in acc]

        z = []
        for m in range(2):
            y = [v for j0 in range(0, NC, JB) for v in mac(m, j0)]
            z.append([y[0]] + [
                (y[j][0] - y[j - 1][1], y[j][1] + y[j - 1][0]) if sgn > 0 else
                (y[j][0] + y[j - 1][1], y[j][1] - y[j - 1][0]) for j in range(1, NC)])
        r = pl.ds(ft * 8, 8)
        wc, ws = tw_ref[0, r, :], tw_ref[1, r, :]
        for j in range(NC):
            (ar, ai), (br, bi) = z[0][j], z[1][j]
            dr, di = ar - br, ai - bi
            for n, val in enumerate((ar + br, ai + bi, dr * wc - di * ws, dr * ws + di * wc)):
                zs[sl][j, pl.ds(n * H + ft * 8, 8), :] = val

    def conv_inv(c, j, sl):
        ye = _dot(inv_ref[...], zs[sl][j, 0:2 * H, :].astype(BF))
        yo = _dot(inv_ref[...], zs[sl][j, 2 * H:, :].astype(BF))

        def store():
            be = pltpu.bitcast(ye.astype(BF).astype(F32), jnp.uint32)
            bo = pltpu.bitcast(yo.astype(BF).astype(F32), jnp.uint32)
            y_v[pl.ds(j * C, C), pl.ds(pl.multiple_of(c * W, W), W)] = (
                pltpu.bitcast((be >> 16) | bo, BF))
        return store

    for cp in (*k_copies, *conv_copies(0)):
        cp.wait()
    for c in range(1, AHEAD):
        for cp in conv_copies(c):
            cp.start()

    for j in range(NC):
        conv_fwd(0, j, 0)()

    def conv_step(c, sl, with_fwd, with_inv=True):
        for j in range(NC):
            sts = []
            if with_fwd:
                sts.append(conv_fwd(c + 1, j, 1 - sl))
            if with_inv:
                sts.append(conv_inv(c - 1, j, 1 - sl))
            conv_mac(sl, j, 1)
            conv_mac(sl, j + NC, -1)
            for st in sts:
                st()

    def feed(c):
        for cp in conv_copies(c + 1):
            cp.wait()

        @pl.when(c + AHEAD < NW)
        def _():
            for cp in conv_copies(jnp.minimum(c + AHEAD, NW - 1)):
                cp.start()

        for n, cp in enumerate(w_copies[:3]):
            pl.when(c == NW - AHEAD + n - 1)(cp.start)

    feed(jnp.int32(0))
    conv_step(0, 0, True, False)

    def conv_block(c, carry):
        for u in range(2):
            feed(2 * c + 1 + u)
            conv_step(2 * c + 1 + u, 1 - u, True)
        return carry

    lax.fori_loop(0, 3, conv_block, 0)
    w_copies[3].start()
    conv_step(NW - 1, (NW - 1) % 2, False)

    for j in range(NC):
        conv_inv(NW - 1, j, (NW - 1) % 2)()

    def blk(v, r=0, n=BM):
        return pl.ds(pl.multiple_of((v % NB) * BM + r, 8), n)

    RP = 64
    NP = BM // RP

    def prep(v, src, p):
        rows = blk(v, p * RP, RP)
        x = src[rows, :].astype(F32)
        x = x + _ln(x) * y_v[rows, :].astype(F32)
        x_v[rows, :] = x
        xn = _ln(x)
        xn_v[rows, :] = xn
        la[v % 2, p * RP:(p + 1) * RP, :] = _ln(xn).astype(BF)

    def shift(v, p):
        Q = D // 4
        for g, sh in enumerate((-1, 1, -2, 2)):
            win = h_v[blk(v, p * RP, RP + 2 * HALO), g * Q:(g + 1) * Q]
            gb[v % 2, p * RP:(p + 1) * RP, g * Q:(g + 1) * Q] = (
                win[HALO + sh:HALO + sh + RP, :].astype(BF))

    def ln1(v, p):
        lb[v % 2, p * RP:(p + 1) * RP, :] = _ln(xn_v[blk(v, p * RP, RP), :]).astype(BF)

    NCH = 256

    def mix_a(v, fill=()):
        for n in range(D // NCH):
            cols = slice(n * NCH, (n + 1) * NCH)
            h_v[blk(v, HALO), cols] = _gelu(_dot(la[v % 2], w1_v[:, cols]))
            for f in fill[n::D // NCH]:
                f()

    def mix_b(v, fill=()):
        for n in range(D // NCH):
            cols = slice(n * NCH, (n + 1) * NCH)
            xn_v[blk(v), cols] = xn_v[blk(v), cols] + _dot(gb[v % 2], w2_v[:, cols])
            for f in fill[n::D // NCH]:
                f()

    def mlp(v, fill=()):
        rows = blk(v)
        h2 = _gelu(_dot(lb[v % 2], w3_v[...])).astype(BF)
        NO = 128
        for n in range(D // NO):
            cols = slice(n * NO, (n + 1) * NO)
            x = x_v[rows, cols] + xn_v[rows, cols] + _dot(h2, w4_v[:, cols])
            x_v[rows, cols] = x
            o_v[rows, cols] = x.astype(BF)
            for f in (fill[n // 2::D // NO // 2] if n % 2 == 0 else ()):
                f()

    def pieces(fn, *args):
        return [functools.partial(fn, *args, p) for p in range(NP)]

    def run(fs):
        for f in fs:
            f()

    def out_copy(v):
        return pltpu.make_async_copy(o_v.at[blk(v), :], o_hbm.at[blk(v), :], sem_o.at[v % NB])

    SK = 6
    q_cp, w1_cp, w2_cp, w3_cp, w4_cp = w_copies
    q_cp.wait()
    x_v[(NB - 1) * BM:, :] = q_v[(NB - 1) * BM:, :].astype(F32)
    run(pieces(prep, 0, q_v))
    w1_cp.wait()
    w4_cp.start()

    def pro(v, carry):
        mix_a(v, pieces(prep, v + 1, q_v))
        return carry

    lax.fori_loop(0, SK, pro, 0)
    w2_cp.wait()
    run(pieces(shift, 0))
    mix_b(0, pieces(shift, 1))
    mix_b(1, pieces(shift, 2) + pieces(ln1, 0))
    w3_cp.wait()
    w4_cp.wait()

    def main(i, carry):
        mix_b(i + 2, pieces(shift, i + 3))
        mix_a(i + SK, pieces(ln1, i + 1))
        mlp(i, pieces(prep, i + SK + 1, x_v))

        @pl.when(i >= NB)
        def _():
            out_copy(i).start()
        return carry

    lax.fori_loop(0, 2 * NB - SK, main, 0)

    def tail(i, carry):
        mix_b(i + 2, pieces(shift, i + 3))
        mlp(i, pieces(ln1, i + 1))
        out_copy(i).start()
        return carry

    lax.fori_loop(2 * NB - SK, 2 * NB - 2, tail, 0)

    def last(i, carry):
        mlp(i, pieces(ln1, i + 1))
        out_copy(i).start()
        return carry

    lax.fori_loop(2 * NB - 2, 2 * NB, last, 0)
    for b in range(NB):
        out_copy(b).wait()


@jax.jit
def pallas_interleave_layers__ssm_conv_h3__mixer_s_mlp__prompt_kernel(
    A_q, A_k, A_v, A_shift_k, A_ssm_k, A_ssm_D, B_x, B_w1, B_w2, B_w3, B_w4,
):
    consts = _dft_mats()
    hbm = pl.BlockSpec(memory_space=pl.ANY)
    vm = pl.BlockSpec(memory_space=pltpu.VMEM)
    out = pl.pallas_call(
        _kernel,
        in_specs=[hbm, hbm, hbm, vm, hbm, vm, hbm, hbm, hbm, hbm, hbm, hbm, hbm, hbm],
        out_specs=hbm,
        out_shape=jax.ShapeDtypeStruct((S, D), BF),
        scratch_shapes=[
            *[pltpu.VMEM(a.shape, a.dtype) for a in consts], pltpu.SemaphoreType.DMA((4,)),
            pltpu.VMEM((S, D), BF), pltpu.VMEM((NW, S + KH, W), BF), pltpu.VMEM((NW, S, W), BF),
            pltpu.VMEM((NW, W, S), BF),
            pltpu.VMEM((D, D), BF), pltpu.VMEM((D, D), BF),
            pltpu.VMEM((D, F), BF), pltpu.VMEM((F, D), BF),
            pltpu.VMEM((NW, 8, W), F32),
            *[pltpu.VMEM((NC, 6 * H, W), F32)] * 4, *[pltpu.VMEM((NC, 4 * H, W), F32)] * 2,
            pltpu.VMEM((S, D), BF), pltpu.VMEM((S, D), F32), pltpu.VMEM((S, D), F32),
            pltpu.VMEM((S + 2 * HALO, D), F32), pltpu.VMEM((S, D), BF),
            pltpu.VMEM((2, BM, D), BF), pltpu.VMEM((2, BM, D), BF), pltpu.VMEM((2, BM, D), BF),
            pltpu.SemaphoreType.DMA((3, NW)), pltpu.SemaphoreType.DMA((5,)),
            pltpu.SemaphoreType.DMA((NB,)),
        ],
        compiler_params=pltpu.CompilerParams(vmem_limit_bytes=120 * 1024 * 1024),
    )(A_q.reshape(S, D), A_k.reshape(S, D), A_v.reshape(S, D), A_shift_k, A_ssm_k,
      A_ssm_D.reshape(1, D), B_w1, B_w2, B_w3, B_w4, *consts)
    return out.reshape(1, S, D)
```

```python
import functools
import numpy as np
import jax
import jax.numpy as jnp
from jax import lax
import jax.experimental.pallas as pl
import jax.experimental.pallas.tpu as pltpu

S, D, F = 2048, 1024, 3584
KS = 4
JB = 8
H = 128
C = 256
NC = S // C
KH = 16
W = 128
NW = D // W
BM = 256
NB = S // BM
HALO = 8
EPS = 1e-5
BF = jnp.bfloat16
F32 = jnp.float32


def _dft_mats():
    f = np.concatenate([np.arange(0, H, 2), np.arange(1, H, 2)])
    th = 2.0 * np.pi * (f + 0.5) / (2 * C)
    ph = th[:, None] * (2 * np.arange(H))[None, :]
    half = np.concatenate([np.cos(ph), -np.sin(ph)], 0)
    inv = np.concatenate([np.cos(ph).T, -np.sin(ph).T], 1) / C
    t = np.arange(C)[None, :]
    lo, hi = th[:, None] * t, (np.pi - th)[:, None] * t
    full = np.concatenate([np.cos(lo), -np.sin(lo), np.cos(hi), np.sin(hi)], 0)
    tw = np.stack([np.cos(th), np.sin(th)])[:, :, None] * np.ones((1, 1, W))
    return (np.asarray(half, dtype=BF), np.asarray(inv, dtype=BF), np.asarray(full, dtype=BF),
            np.asarray(tw, dtype=np.float32))


def _ln(x):
    m = jnp.mean(x, axis=-1, keepdims=True)
    d = x - m
    v = jnp.mean(d * d, axis=-1, keepdims=True)
    return d * lax.rsqrt(v + EPS)


def _gelu(x):
    c0 = 0.7978845608028654
    u = x * (x * x * (c0 * 0.044715) + c0)
    hx = 0.5 * x
    return hx * jnp.tanh(u) + hx


def _dot(a, b):
    return jnp.dot(a, b, preferred_element_type=F32)


def _kernel(q_hbm, k_hbm, v_hbm, sk_ref, kk_hbm, d_ref, w1_hbm, w2_hbm, w3_hbm, w4_hbm,
            half_hbm, inv_hbm, full_hbm, tw_hbm, o_hbm,
            half_ref, inv_ref, full_ref, tw_ref, sem_k,
            q_v, k_v, v_v, kk_v, w1_v, w2_v, w3_v, w4_v,
            taps, xs0, xs1, ks0, ks1, zs0, zs1, y_v, x_v, xn_v, h_v, o_v, la, lb, gb, sem_c, sem_w, sem_o):

    xs, ks, zs = (xs0, xs1), (ks0, ks1), (zs0, zs1)

    def conv_copies(c):
        cols = pl.ds(pl.multiple_of(c * W, W), W)
        return (
            pltpu.make_async_copy(k_hbm.at[:, cols], k_v.at[c, pl.ds(KH, S), :], sem_c.at[0, c]),
            pltpu.make_async_copy(v_hbm.at[:, cols], v_v.at[c], sem_c.at[1, c]),
            pltpu.make_async_copy(kk_hbm.at[cols, :], kk_v.at[c], sem_c.at[2, c]),
        )

    w_copies = [
        pltpu.make_async_copy(q_hbm, q_v, sem_w.at[0]),
        pltpu.make_async_copy(w1_hbm, w1_v, sem_w.at[1]),
        pltpu.make_async_copy(w2_hbm, w2_v, sem_w.at[2]),
        pltpu.make_async_copy(w3_hbm, w3_v, sem_w.at[3]),
        pltpu.make_async_copy(w4_hbm, w4_v, sem_w.at[4]),
    ]
    k_copies = [pltpu.make_async_copy(a, b, sem_k.at[n]) for n, (a, b) in enumerate(
        ((half_hbm, half_ref), (inv_hbm, inv_ref), (full_hbm, full_ref), (tw_hbm, tw_ref)))]
    for cp in k_copies:
        cp.start()
    AHEAD = 3
    for c in range(1):
        for cp in conv_copies(c):
            cp.start()

    for c in range(NW):
        k_v[c, 0:KH, :] = jnp.zeros((KH, W), BF)
        taps[c, 0:KS, :] = sk_ref[:, c * W:(c + 1) * W].astype(F32)
        taps[c, KS:KS + 1, :] = d_ref[...].astype(F32).reshape(1, D)[:, c * W:(c + 1) * W]
    h_v[0:HALO, :] = jnp.zeros((HALO, D), F32)
    h_v[HALO + S:, :] = jnp.zeros((HALO, D), F32)

    def even_odd(x):
        u = pltpu.bitcast(x, jnp.uint32)
        return (pltpu.bitcast(u << 16, F32), pltpu.bitcast(u & jnp.uint32(0xFFFF0000), F32))

    def conv_fwd(c, j, sl):
        tp = taps[c]
        t = [tp[d:d + 1, :] for d in range(KS)]
        ke, ko = even_odd(k_v[c, pl.ds(j * C, C + KH), :])
        ve, vo = even_odd(v_v[c, pl.ds(j * C, C), :])
        P = KH // 2
        ke0, ke1 = ke[P:], ke[P - 1:P - 1 + H]
        ko0, ko1, ko2 = ko[P:], ko[P - 1:P - 1 + H], ko[P - 2:P - 2 + H]
        kve = (ke0 * t[0] + ko1 * t[1] + ke1 * t[2] + ko2 * t[3]) * ve
        kvo = (ko0 * t[0] + ke0 * t[1] + ko1 * t[2] + ke1 * t[3]) * vo
        ef = _dot(half_ref[...], kve.astype(BF))
        of = _dot(half_ref[...], kvo.astype(BF))
        kf = lax.dot_general(full_ref[...], kk_v[c, :, pl.ds(j * C, C)],
                             (((1,), (1,)), ((), ())), preferred_element_type=F32)

        def store():
            wc, ws = tw_ref[0], tw_ref[1]
            pr = of[:H] * wc + of[H:] * ws
            pi = of[H:] * wc - of[:H] * ws
            for m, (xr, xi) in enumerate(((ef[:H] + pr, ef[H:] + pi), (ef[:H] - pr, ef[H:] - pi))):
                kr, ki = kf[2 * m * H:(2 * m + 1) * H], kf[(2 * m + 1) * H:(2 * m + 2) * H]
                if j == 0:
                    kr = kr + tp[KS:KS + 1, :]
                for n, (xv, kv) in enumerate(((xr, ki - kr), (xi, ki + kr), (xr + xi, kr))):
                    xs[sl][j, pl.ds((3 * m + n) * H, H), :] = xv
                    ks[sl][j, pl.ds((3 * m + n) * H, H), :] = kv
        return store

    def conv_mac(sl, ft, sgn):
        def mac(m, j0):
            acc = [[None] * 3 for _ in range(JB)]
            for i in range(j0 + JB):
                for n in range(3):
                    r = pl.ds((3 * m + n) * H + ft * 8, 8)
                    xv = xs[sl][i, r, :]
                    for u in range(JB):
                        if j0 + u >= i:
                            p = xv * ks[sl][j0 + u - i, r, :]
                            acc[u][n] = p if acc[u][n] is None else acc[u][n] + p
            return [(a[2] - a[1], a[2] + a[0]) for a in acc]

        z = []
        for m in range(2):
            y = [v for j0 in range(0, NC, JB) for v in mac(m, j0)]
            z.append([y[0]] + [
                (y[j][0] - y[j - 1][1], y[j][1] + y[j - 1][0]) if sgn > 0 else
                (y[j][0] + y[j - 1][1], y[j][1] - y[j - 1][0]) for j in range(1, NC)])
        r = pl.ds(ft * 8, 8)
        wc, ws = tw_ref[0, r, :], tw_ref[1, r, :]
        for j in range(NC):
            (ar, ai), (br, bi) = z[0][j], z[1][j]
            dr, di = ar - br, ai - bi
            for n, val in enumerate((ar + br, ai + bi, dr * wc - di * ws, dr * ws + di * wc)):
                zs[sl][j, pl.ds(n * H + ft * 8, 8), :] = val

    def conv_inv(c, j, sl):
        ye = _dot(inv_ref[...], zs[sl][j, 0:2 * H, :].astype(BF))
        yo = _dot(inv_ref[...], zs[sl][j, 2 * H:, :].astype(BF))

        def store():
            be = pltpu.bitcast(ye.astype(BF).astype(F32), jnp.uint32)
            bo = pltpu.bitcast(yo.astype(BF).astype(F32), jnp.uint32)
            y_v[pl.ds(j * C, C), pl.ds(pl.multiple_of(c * W, W), W)] = (
                pltpu.bitcast((be >> 16) | bo, BF))
        return store

    for cp in (*k_copies, *conv_copies(0)):
        cp.wait()
    for c in range(1, AHEAD):
        for cp in conv_copies(c):
            cp.start()

    for j in range(NC):
        conv_fwd(0, j, 0)()

    def conv_step(c, sl, with_fwd, with_inv=True):
        for j in range(NC):
            sts = []
            if with_fwd:
                sts.append(conv_fwd(c + 1, j, 1 - sl))
            if with_inv:
                sts.append(conv_inv(c - 1, j, 1 - sl))
            conv_mac(sl, j, 1)
            conv_mac(sl, j + NC, -1)
            for st in sts:
                st()

    def feed(c):
        for cp in conv_copies(c + 1):
            cp.wait()

        @pl.when(c + AHEAD < NW)
        def _():
            for cp in conv_copies(jnp.minimum(c + AHEAD, NW - 1)):
                cp.start()

        for n, cp in enumerate(w_copies[:3]):
            pl.when(c == NW - AHEAD + n - 1)(cp.start)

    feed(jnp.int32(0))
    conv_step(0, 0, True, False)

    def conv_block(c, carry):
        for u in range(2):
            feed(2 * c + 1 + u)
            conv_step(2 * c + 1 + u, 1 - u, True)
        return carry

    lax.fori_loop(0, 3, conv_block, 0)
    w_copies[3].start()
    conv_step(NW - 1, (NW - 1) % 2, False)

    for j in range(NC):
        conv_inv(NW - 1, j, (NW - 1) % 2)()

    def blk(v, r=0, n=BM):
        return pl.ds(pl.multiple_of((v % NB) * BM + r, 8), n)

    RP = 64
    NP = BM // RP

    def prep(v, src, p):
        rows = blk(v, p * RP, RP)
        x = src[rows, :].astype(F32)
        x = x + _ln(x) * y_v[rows, :].astype(F32)
        x_v[rows, :] = x
        xn = _ln(x)
        xn_v[rows, :] = xn
        la[v % 2, p * RP:(p + 1) * RP, :] = _ln(xn).astype(BF)

    def shift(v, p):
        Q = D // 4
        for g, sh in enumerate((-1, 1, -2, 2)):
            win = h_v[blk(v, p * RP, RP + 2 * HALO), g * Q:(g + 1) * Q]
            gb[v % 2, p * RP:(p + 1) * RP, g * Q:(g + 1) * Q] = (
                win[HALO + sh:HALO + sh + RP, :].astype(BF))

    def ln1(v, p):
        lb[v % 2, p * RP:(p + 1) * RP, :] = _ln(xn_v[blk(v, p * RP, RP), :]).astype(BF)

    NCH = 256

    def mix_a(v, fill=()):
        for n in range(D // NCH):
            cols = slice(n * NCH, (n + 1) * NCH)
            h_v[blk(v, HALO), cols] = _gelu(_dot(la[v % 2], w1_v[:, cols]))
            for f in fill[n::D // NCH]:
                f()

    def mix_b(v, fill=()):
        for n in range(D // NCH):
            cols = slice(n * NCH, (n + 1) * NCH)
            xn_v[blk(v), cols] = xn_v[blk(v), cols] + _dot(gb[v % 2], w2_v[:, cols])
            for f in fill[n::D // NCH]:
                f()

    def mlp(v, fill=()):
        rows = blk(v)
        h2 = _gelu(_dot(lb[v % 2], w3_v[...])).astype(BF)
        NO = 128
        for n in range(D // NO):
            cols = slice(n * NO, (n + 1) * NO)
            x = x_v[rows, cols] + xn_v[rows, cols] + _dot(h2, w4_v[:, cols])
            x_v[rows, cols] = x
            o_v[rows, cols] = x.astype(BF)
            for f in (fill[n // 2::D // NO // 2] if n % 2 == 0 else ()):
                f()

    def pieces(fn, *args):
        return [functools.partial(fn, *args, p) for p in range(NP)]

    def run(fs):
        for f in fs:
            f()

    def out_copy(v):
        return pltpu.make_async_copy(o_v.at[blk(v), :], o_hbm.at[blk(v), :], sem_o.at[v % NB])

    SK = 6
    q_cp, w1_cp, w2_cp, w3_cp, w4_cp = w_copies
    q_cp.wait()
    x_v[(NB - 1) * BM:, :] = q_v[(NB - 1) * BM:, :].astype(F32)
    run(pieces(prep, 0, q_v))
    w1_cp.wait()
    w4_cp.start()

    def pro(v, carry):
        mix_a(v, pieces(prep, v + 1, q_v))
        return carry

    lax.fori_loop(0, SK, pro, 0)
    w2_cp.wait()
    run(pieces(shift, 0))
    mix_b(0, pieces(shift, 1))
    mix_b(1, pieces(shift, 2) + pieces(ln1, 0))
    w3_cp.wait()
    w4_cp.wait()

    def main(i, carry):
        mix_b(i + 2, pieces(shift, i + 3))
        mix_a(i + SK, pieces(ln1, i + 1))
        mlp(i, pieces(prep, i + SK + 1, x_v))

        @pl.when(i >= NB)
        def _():
            out_copy(i).start()
        return carry

    lax.fori_loop(0, 2 * NB - SK, main, 0)

    def tail(i, carry):
        mix_b(i + 2, pieces(shift, i + 3))
        mlp(i, pieces(ln1, i + 1))
        out_copy(i).start()
        return carry

    lax.fori_loop(2 * NB - SK, 2 * NB - 2, tail, 0)

    def last(i, carry):
        mlp(i, pieces(ln1, i + 1))
        out_copy(i).start()
        return carry

    lax.fori_loop(2 * NB - 2, 2 * NB, last, 0)
    for b in range(NB):
        out_copy(b).wait()


@jax.jit
def pallas_interleave_layers__ssm_conv_h3__mixer_s_mlp__prompt_kernel(
    A_q, A_k, A_v, A_shift_k, A_ssm_k, A_ssm_D, B_x, B_w1, B_w2, B_w3, B_w4,
):
    consts = _dft_mats()
    hbm = pl.BlockSpec(memory_space=pl.ANY)
    vm = pl.BlockSpec(memory_space=pltpu.VMEM)
    out = pl.pallas_call(
        _kernel,
        in_specs=[hbm, hbm, hbm, vm, hbm, vm, hbm, hbm, hbm, hbm, hbm, hbm, hbm, hbm],
        out_specs=hbm,
        out_shape=jax.ShapeDtypeStruct((S, D), BF),
        scratch_shapes=[
            *[pltpu.VMEM(a.shape, a.dtype) for a in consts], pltpu.SemaphoreType.DMA((4,)),
            pltpu.VMEM((S, D), BF), pltpu.VMEM((NW, S + KH, W), BF), pltpu.VMEM((NW, S, W), BF),
            pltpu.VMEM((NW, W, S), BF),
            pltpu.VMEM((D, D), BF), pltpu.VMEM((D, D), BF),
            pltpu.VMEM((D, F), BF), pltpu.VMEM((F, D), BF),
            pltpu.VMEM((NW, 8, W), F32),
            *[pltpu.VMEM((NC, 6 * H, W), F32)] * 4, *[pltpu.VMEM((NC, 4 * H, W), F32)] * 2,
            pltpu.VMEM((S, D), BF), pltpu.VMEM((S, D), F32), pltpu.VMEM((S, D), F32),
            pltpu.VMEM((S + 2 * HALO, D), F32), pltpu.VMEM((S, D), BF),
            pltpu.VMEM((2, BM, D), BF), pltpu.VMEM((2, BM, D), BF), pltpu.VMEM((2, BM, D), BF),
            pltpu.SemaphoreType.DMA((3, NW)), pltpu.SemaphoreType.DMA((5,)),
            pltpu.SemaphoreType.DMA((NB,)),
        ],
        compiler_params=pltpu.CompilerParams(vmem_limit_bytes=120 * 1024 * 1024),
    )(A_q.reshape(S, D), A_k.reshape(S, D), A_v.reshape(S, D), A_shift_k.T, A_ssm_k,
      A_ssm_D, B_w1, B_w2, B_w3, B_w4, *consts)
    return out.reshape(1, S, D)
```

```python
import functools
import numpy as np
import jax
import jax.numpy as jnp
from jax import lax
import jax.experimental.pallas as pl
import jax.experimental.pallas.tpu as pltpu

S, D, F = 2048, 1024, 3584
KS = 4
JB = 8
H = 128
C = 256
NC = S // C
KH = 16
W = 128
NW = D // W
BM = 256
NB = S // BM
HALO = 8
EPS = 1e-5
BF = jnp.bfloat16
F32 = jnp.float32


def _dft_mats():
    f = np.concatenate([np.arange(0, H, 2), np.arange(1, H, 2)])
    th = 2.0 * np.pi * (f + 0.5) / (2 * C)
    ph = th[:, None] * (2 * np.arange(H))[None, :]
    half = np.concatenate([np.cos(ph), -np.sin(ph)], 0)
    inv = np.concatenate([np.cos(ph).T, -np.sin(ph).T], 1) / C
    t = np.arange(C)[None, :]
    lo, hi = th[:, None] * t, (np.pi - th)[:, None] * t
    full = np.concatenate([np.cos(lo), -np.sin(lo), np.cos(hi), np.sin(hi)], 0)
    tw = np.stack([np.cos(th), np.sin(th)])[:, :, None] * np.ones((1, 1, W))
    return (np.asarray(half, dtype=BF), np.asarray(inv, dtype=BF), np.asarray(full, dtype=BF),
            np.asarray(tw, dtype=np.float32))


def _ln(x):
    m = jnp.mean(x, axis=-1, keepdims=True)
    d = x - m
    v = jnp.mean(d * d, axis=-1, keepdims=True)
    return d * lax.rsqrt(v + EPS)


def _gelu(x):
    c0 = 0.7978845608028654
    u = x * (x * x * (c0 * 0.044715) + c0)
    hx = 0.5 * x
    return hx * jnp.tanh(u) + hx


def _dot(a, b):
    return jnp.dot(a, b, preferred_element_type=F32)


def _kernel(q_hbm, k_hbm, v_hbm, sk_ref, kk_hbm, d_ref, w1_hbm, w2_hbm, w3_hbm, w4_hbm,
            half_hbm, inv_hbm, full_hbm, tw_hbm, z_ref, o_hbm,
            half_ref, inv_ref, full_ref, tw_ref, sem_k,
            q_v, k_v, v_v, kk_v, w1_v, w2_v, w3_v, w4_v,
            taps, xs0, xs1, ks0, ks1, zs0, zs1, y_v, x_v, xn_v, h_v, o_v, la, lb, gb, sem_c, sem_w, sem_o):

    xs, ks, zs = (xs0, xs1), (ks0, ks1), (zs0, zs1)

    def conv_copies(c):
        cols = pl.ds(pl.multiple_of(c * W, W), W)
        return (
            pltpu.make_async_copy(k_hbm.at[:, cols], k_v.at[c, pl.ds(KH, S), :], sem_c.at[0, c]),
            pltpu.make_async_copy(v_hbm.at[:, cols], v_v.at[c], sem_c.at[1, c]),
            pltpu.make_async_copy(kk_hbm.at[cols, :], kk_v.at[c], sem_c.at[2, c]),
        )

    w_copies = [
        pltpu.make_async_copy(q_hbm, q_v, sem_w.at[0]),
        pltpu.make_async_copy(w1_hbm, w1_v, sem_w.at[1]),
        pltpu.make_async_copy(w2_hbm, w2_v, sem_w.at[2]),
        pltpu.make_async_copy(w3_hbm, w3_v, sem_w.at[3]),
        pltpu.make_async_copy(w4_hbm, w4_v, sem_w.at[4]),
    ]
    k_copies = [pltpu.make_async_copy(a, b, sem_k.at[n]) for n, (a, b) in enumerate(
        ((half_hbm, half_ref), (inv_hbm, inv_ref), (full_hbm, full_ref), (tw_hbm, tw_ref)))]
    for cp in k_copies:
        cp.start()
    AHEAD = 3
    for c in range(1):
        for cp in conv_copies(c):
            cp.start()

    for c in range(NW):
        k_v[c, 0:KH, :] = jnp.zeros((KH, W), BF)
        taps[c, 0:KS, :] = sk_ref[:, c * W:(c + 1) * W].astype(F32)
        taps[c, KS:KS + 1, :] = d_ref[...].astype(F32).reshape(1, D)[:, c * W:(c + 1) * W]
    h_v[0:HALO, :] = jnp.zeros((HALO, D), F32)
    h_v[HALO + S:, :] = jnp.zeros((HALO, D), F32)

    def even_odd(x):
        u = pltpu.bitcast(x, jnp.uint32)
        return (pltpu.bitcast(u << 16, F32), pltpu.bitcast(u & jnp.uint32(0xFFFF0000), F32))

    def conv_fwd(c, j, sl):
        tp = taps[c]
        t = [tp[d:d + 1, :] for d in range(KS)]
        ke, ko = even_odd(k_v[c, pl.ds(j * C, C + KH), :])
        ve, vo = even_odd(v_v[c, pl.ds(j * C, C), :])
        P = KH // 2
        ke0, ke1 = ke[P:], ke[P - 1:P - 1 + H]
        ko0, ko1, ko2 = ko[P:], ko[P - 1:P - 1 + H], ko[P - 2:P - 2 + H]
        kve = (ke0 * t[0] + ko1 * t[1] + ke1 * t[2] + ko2 * t[3]) * ve
        kvo = (ko0 * t[0] + ke0 * t[1] + ko1 * t[2] + ke1 * t[3]) * vo
        ef = _dot(half_ref[...], kve.astype(BF))
        of = _dot(half_ref[...], kvo.astype(BF))
        kf = lax.dot_general(full_ref[...], kk_v[c, :, pl.ds(j * C, C)],
                             (((1,), (1,)), ((), ())), preferred_element_type=F32)

        def store():
            wc, ws = tw_ref[0], tw_ref[1]
            pr = of[:H] * wc + of[H:] * ws
            pi = of[H:] * wc - of[:H] * ws
            for m, (xr, xi) in enumerate(((ef[:H] + pr, ef[H:] + pi), (ef[:H] - pr, ef[H:] - pi))):
                kr, ki = kf[2 * m * H:(2 * m + 1) * H], kf[(2 * m + 1) * H:(2 * m + 2) * H]
                if j == 0:
                    kr = kr + tp[KS:KS + 1, :]
                for n, (xv, kv) in enumerate(((xr, ki - kr), (xi, ki + kr), (xr + xi, kr))):
                    xs[sl][j, pl.ds((3 * m + n) * H, H), :] = xv
                    ks[sl][j, pl.ds((3 * m + n) * H, H), :] = kv
        return store, [(ef, 3), (of, 3), (kf, 12)]

    def conv_mac(sl, ft, sgn, tie):
        def mac(m, j0):
            acc = [[None] * 3 for _ in range(JB)]
            for n in range(3):
                r = pl.ds((3 * m + n) * H + ft * 8, 8)
                for i in range(j0 + JB):
                    xv = tie(xs[sl][i, r, :])
                    for u in range(JB):
                        if j0 + u >= i:
                            p = xv * ks[sl][j0 + u - i, r, :]
                            acc[u][n] = p if acc[u][n] is None else acc[u][n] + p
            return [(a[2] - a[1], a[2] + a[0]) for a in acc]

        z = []
        for m in range(2):
            y = [v for j0 in range(0, NC, JB) for v in mac(m, j0)]
            z.append([y[0]] + [
                (y[j][0] - y[j - 1][1], y[j][1] + y[j - 1][0]) if sgn > 0 else
                (y[j][0] + y[j - 1][1], y[j][1] - y[j - 1][0]) for j in range(1, NC)])
        r = pl.ds(ft * 8, 8)
        wc, ws = tw_ref[0, r, :], tw_ref[1, r, :]
        for j in range(NC):
            (ar, ai), (br, bi) = z[0][j], z[1][j]
            dr, di = ar - br, ai - bi
            for n, val in enumerate((ar + br, ai + bi, dr * wc - di * ws, dr * ws + di * wc)):
                zs[sl][j, pl.ds(n * H + ft * 8, 8), :] = val

    def conv_inv(c, j, sl):
        ye = _dot(inv_ref[...], zs[sl][j, 0:2 * H, :].astype(BF))
        yo = _dot(inv_ref[...], zs[sl][j, 2 * H:, :].astype(BF))

        def store():
            be = pltpu.bitcast(ye.astype(BF).astype(F32), jnp.uint32)
            bo = pltpu.bitcast(yo.astype(BF).astype(F32), jnp.uint32)
            y_v[pl.ds(j * C, C), pl.ds(pl.multiple_of(c * W, W), W)] = (
                pltpu.bitcast((be >> 16) | bo, BF))
        return store, [(ye, 3), (yo, 3)]

    for cp in (*k_copies, *conv_copies(0)):
        cp.wait()
    for c in range(1, AHEAD):
        for cp in conv_copies(c):
            cp.start()

    for j in range(NC):
        conv_fwd(0, j, 0)[0]()

    def conv_step(c, sl, with_fwd, with_inv=True):
        for j in range(NC):
            sts = []
            if with_fwd:
                sts.append(conv_fwd(c + 1, j, 1 - sl))
            if with_inv:
                sts.append(conv_inv(c - 1, j, 1 - sl))
            never = jnp.full((8, W), z_ref[0], jnp.int32) != 0
            outs = [o for st in sts for o in st[1]]
            need = 2 * 2 * 3 * NC
            tot = sum(w for _, w in outs)
            anchors = []
            for val, w in outs:
                cnt = need * w // tot
                nv = val.shape[0] // 8
                anchors += [val[8 * (t * nv // cnt):8 * (t * nv // cnt) + 8] for t in range(cnt)]
            it = iter(anchors)
            tie = lambda xv: jnp.where(never, next(it), xv)
            conv_mac(sl, j, 1, tie)
            conv_mac(sl, j + NC, -1, tie)
            for st in sts:
                st[0]()

    def feed(c):
        for cp in conv_copies(c + 1):
            cp.wait()

        @pl.when(c + AHEAD < NW)
        def _():
            for cp in conv_copies(jnp.minimum(c + AHEAD, NW - 1)):
                cp.start()

        for n, cp in enumerate(w_copies[:3]):
            pl.when(c == NW - AHEAD + n - 1)(cp.start)

    feed(jnp.int32(0))
    conv_step(0, 0, True, False)

    def conv_block(c, carry):
        for u in range(2):
            feed(2 * c + 1 + u)
            conv_step(2 * c + 1 + u, 1 - u, True)
        return carry

    lax.fori_loop(0, 3, conv_block, 0)
    w_copies[3].start()
    conv_step(NW - 1, (NW - 1) % 2, False)

    for j in range(NC):
        conv_inv(NW - 1, j, (NW - 1) % 2)[0]()

    def blk(v, r=0, n=BM):
        return pl.ds(pl.multiple_of((v % NB) * BM + r, 8), n)

    RP = 64
    NP = BM // RP

    def prep(v, src, p):
        rows = blk(v, p * RP, RP)
        x = src[rows, :].astype(F32)
        x = x + _ln(x) * y_v[rows, :].astype(F32)
        x_v[rows, :] = x
        xn = _ln(x)
        xn_v[rows, :] = xn
        la[v % 2, p * RP:(p + 1) * RP, :] = _ln(xn).astype(BF)

    def shift(v, p):
        Q = D // 4
        for g, sh in enumerate((-1, 1, -2, 2)):
            win = h_v[blk(v, p * RP, RP + 2 * HALO), g * Q:(g + 1) * Q]
            gb[v % 2, p * RP:(p + 1) * RP, g * Q:(g + 1) * Q] = (
                win[HALO + sh:HALO + sh + RP, :].astype(BF))

    def ln1(v, p):
        lb[v % 2, p * RP:(p + 1) * RP, :] = _ln(xn_v[blk(v, p * RP, RP), :]).astype(BF)

    NCH = 256

    def mix_a(v, fill=()):
        for n in range(D // NCH):
            cols = slice(n * NCH, (n + 1) * NCH)
            h_v[blk(v, HALO), cols] = _gelu(_dot(la[v % 2], w1_v[:, cols]))
            for f in fill[n::D // NCH]:
                f()

    def mix_b(v, fill=()):
        for n in range(D // NCH):
            cols = slice(n * NCH, (n + 1) * NCH)
            xn_v[blk(v), cols] = xn_v[blk(v), cols] + _dot(gb[v % 2], w2_v[:, cols])
            for f in fill[n::D // NCH]:
                f()

    def mlp(v, fill=()):
        rows = blk(v)
        h2 = _gelu(_dot(lb[v % 2], w3_v[...])).astype(BF)
        NO = 128
        for n in range(D // NO):
            cols = slice(n * NO, (n + 1) * NO)
            x = x_v[rows, cols] + xn_v[rows, cols] + _dot(h2, w4_v[:, cols])
            x_v[rows, cols] = x
            o_v[rows, cols] = x.astype(BF)
            for f in (fill[n // 2::D // NO // 2] if n % 2 == 0 else ()):
                f()

    def pieces(fn, *args):
        return [functools.partial(fn, *args, p) for p in range(NP)]

    def run(fs):
        for f in fs:
            f()

    def out_copy(v):
        return pltpu.make_async_copy(o_v.at[blk(v), :], o_hbm.at[blk(v), :], sem_o.at[v % NB])

    SK = 6
    q_cp, w1_cp, w2_cp, w3_cp, w4_cp = w_copies
    q_cp.wait()
    x_v[(NB - 1) * BM:, :] = q_v[(NB - 1) * BM:, :].astype(F32)
    run(pieces(prep, 0, q_v))
    w1_cp.wait()
    w4_cp.start()

    def pro(v, carry):
        mix_a(v, pieces(prep, v + 1, q_v))
        return carry

    lax.fori_loop(0, SK, pro, 0)
    w2_cp.wait()
    run(pieces(shift, 0))
    mix_b(0, pieces(shift, 1))
    mix_b(1, pieces(shift, 2) + pieces(ln1, 0))
    w3_cp.wait()
    w4_cp.wait()

    def main(i, carry):
        mix_b(i + 2, pieces(shift, i + 3))
        mix_a(i + SK, pieces(ln1, i + 1))
        mlp(i, pieces(prep, i + SK + 1, x_v))

        @pl.when(i >= NB)
        def _():
            out_copy(i).start()
        return carry

    lax.fori_loop(0, 2 * NB - SK, main, 0)

    def tail(i, carry):
        mix_b(i + 2, pieces(shift, i + 3))
        mlp(i, pieces(ln1, i + 1))
        out_copy(i).start()
        return carry

    lax.fori_loop(2 * NB - SK, 2 * NB - 2, tail, 0)

    def last(i, carry):
        mlp(i, pieces(ln1, i + 1))
        out_copy(i).start()
        return carry

    lax.fori_loop(2 * NB - 2, 2 * NB, last, 0)
    for b in range(NB):
        out_copy(b).wait()


@jax.jit
def pallas_interleave_layers__ssm_conv_h3__mixer_s_mlp__prompt_kernel(
    A_q, A_k, A_v, A_shift_k, A_ssm_k, A_ssm_D, B_x, B_w1, B_w2, B_w3, B_w4,
):
    consts = _dft_mats()
    hbm = pl.BlockSpec(memory_space=pl.ANY)
    vm = pl.BlockSpec(memory_space=pltpu.VMEM)
    out = pl.pallas_call(
        _kernel,
        in_specs=[hbm, hbm, hbm, vm, hbm, vm, hbm, hbm, hbm, hbm, hbm, hbm, hbm, hbm, pl.BlockSpec(memory_space=pltpu.SMEM)],
        out_specs=hbm,
        out_shape=jax.ShapeDtypeStruct((S, D), BF),
        scratch_shapes=[
            *[pltpu.VMEM(a.shape, a.dtype) for a in consts], pltpu.SemaphoreType.DMA((4,)),
            pltpu.VMEM((S, D), BF), pltpu.VMEM((NW, S + KH, W), BF), pltpu.VMEM((NW, S, W), BF),
            pltpu.VMEM((NW, W, S), BF),
            pltpu.VMEM((D, D), BF), pltpu.VMEM((D, D), BF),
            pltpu.VMEM((D, F), BF), pltpu.VMEM((F, D), BF),
            pltpu.VMEM((NW, 8, W), F32),
            *[pltpu.VMEM((NC, 6 * H, W), F32)] * 4, *[pltpu.VMEM((NC, 4 * H, W), F32)] * 2,
            pltpu.VMEM((S, D), BF), pltpu.VMEM((S, D), F32), pltpu.VMEM((S, D), F32),
            pltpu.VMEM((S + 2 * HALO, D), F32), pltpu.VMEM((S, D), BF),
            pltpu.VMEM((2, BM, D), BF), pltpu.VMEM((2, BM, D), BF), pltpu.VMEM((2, BM, D), BF),
            pltpu.SemaphoreType.DMA((3, NW)), pltpu.SemaphoreType.DMA((5,)),
            pltpu.SemaphoreType.DMA((NB,)),
        ],
        compiler_params=pltpu.CompilerParams(vmem_limit_bytes=120 * 1024 * 1024),
    )(A_q.reshape(S, D), A_k.reshape(S, D), A_v.reshape(S, D), A_shift_k.T, A_ssm_k,
      A_ssm_D, B_w1, B_w2, B_w3, B_w4, *consts, np.zeros((1,), np.int32))
    return out.reshape(1, S, D)
```

```python
import numpy as np
import jax
import jax.numpy as jnp
from jax import lax
import jax.experimental.pallas as pl
import jax.experimental.pallas.tpu as pltpu

S, D, F = 2048, 1024, 3584
GAP = 14
KS = 4
JB = 8
H = 128
C = 256
NC = S // C
KH = 16
W = 128
NW = D // W
BM = 256
NB = S // BM
HALO = 8
EPS = 1e-5
BF = jnp.bfloat16
F32 = jnp.float32


def _dft_mats():
    f = np.concatenate([np.arange(0, H, 2), np.arange(1, H, 2)])
    th = 2.0 * np.pi * (f + 0.5) / (2 * C)
    ph = th[:, None] * (2 * np.arange(H))[None, :]
    half = np.concatenate([np.cos(ph), -np.sin(ph)], 0)
    inv = np.concatenate([np.cos(ph).T, -np.sin(ph).T], 1) / C
    t = np.arange(C)[None, :]
    lo, hi = th[:, None] * t, (np.pi - th)[:, None] * t
    full = np.concatenate([np.cos(lo), -np.sin(lo), np.cos(hi), np.sin(hi)], 0)
    tw = np.stack([np.cos(th), np.sin(th)])[:, :, None] * np.ones((1, 1, W))

    def pack(a):
        u = np.asarray(a, dtype=BF).view(np.uint16).astype(np.uint32)
        return u[0::2] | (u[1::2] << 16)

    return pack(half), pack(inv), pack(full), np.asarray(tw, dtype=np.float32)


def _ln(x):
    m = jnp.mean(x, axis=-1, keepdims=True)
    d = x - m
    v = jnp.mean(d * d, axis=-1, keepdims=True)
    return d * lax.rsqrt(v + EPS)


def _gelu(x):
    c0 = 0.7978845608028654
    u = x * (x * x * (c0 * 0.044715) + c0)
    hx = 0.5 * x
    return hx * jnp.tanh(u) + hx


def _dot(a, b):
    return jnp.dot(a, b, preferred_element_type=F32)


def _kernel(q_hbm, k_hbm, v_hbm, sk_ref, kk_hbm, d_ref, w1_hbm, w2_hbm, w3_hbm, w4_hbm,
            half_hbm, inv_hbm, full_hbm, tw_hbm, z_ref, o_hbm,
            half_ref, inv_ref, full_ref, tw_ref, sem_k,
            q_v, k_v, v_v, kk_v, w1_v, w2_v, w3_v, w4_v,
            taps, xs0, xs1, ks0, ks1, zs0, zs1, y_v, x_v, xn_v, h_v, o_v, la, lb, gb, sem_c, sem_w, sem_o):

    xs, ks, zs = (xs0, xs1), (ks0, ks1), (zs0, zs1)

    def conv_copies(c):
        cols = pl.ds(pl.multiple_of(c * W, W), W)
        return (
            pltpu.make_async_copy(k_hbm.at[:, cols], k_v.at[c, pl.ds(KH, S), :], sem_c.at[0, c]),
            pltpu.make_async_copy(v_hbm.at[:, cols], v_v.at[c], sem_c.at[1, c]),
            pltpu.make_async_copy(kk_hbm.at[cols, :], kk_v.at[c], sem_c.at[2, c]),
        )

    w_copies = [
        pltpu.make_async_copy(q_hbm, q_v, sem_w.at[0]),
        pltpu.make_async_copy(w1_hbm, w1_v, sem_w.at[1]),
        pltpu.make_async_copy(w2_hbm, w2_v, sem_w.at[2]),
        pltpu.make_async_copy(w3_hbm, w3_v, sem_w.at[3]),
        pltpu.make_async_copy(w4_hbm, w4_v, sem_w.at[4]),
    ]
    k_copies = [pltpu.make_async_copy(a, b, sem_k.at[n]) for n, (a, b) in enumerate(
        ((half_hbm, half_ref), (inv_hbm, inv_ref), (full_hbm, full_ref), (tw_hbm, tw_ref)))]
    for cp in k_copies:
        cp.start()
    AHEAD = 3
    for c in range(1):
        for cp in conv_copies(c):
            cp.start()

    for c in range(NW):
        k_v[c, 0:KH, :] = jnp.zeros((KH, W), BF)
        taps[c] = jnp.zeros((8, W), F32)
        taps[c, 0:KS, :] = sk_ref[:, c * W:(c + 1) * W].astype(F32)
        taps[c, KS:KS + 1, :] = d_ref[...].astype(F32).reshape(1, D)[:, c * W:(c + 1) * W]
    h_v[0:HALO, :] = jnp.zeros((HALO, D), F32)
    h_v[HALO + S:, :] = jnp.zeros((HALO, D), F32)

    def even_odd(x):
        u = pltpu.bitcast(x, jnp.uint32)
        return (pltpu.bitcast(u << 16, F32), pltpu.bitcast(u & jnp.uint32(0xFFFF0000), F32))

    def conv_fwd(c, j, sl):
        tp = taps[c]
        t = [tp[d:d + 1, :] for d in range(KS)]
        ke, ko = even_odd(k_v[c, pl.ds(j * C, C + KH), :])
        ve, vo = even_odd(v_v[c, pl.ds(j * C, C), :])
        P = KH // 2
        ke0, ke1 = ke[P:], ke[P - 1:P - 1 + H]
        ko0, ko1, ko2 = ko[P:], ko[P - 1:P - 1 + H], ko[P - 2:P - 2 + H]
        kve = (ke0 * t[0] + ko1 * t[1] + ke1 * t[2] + ko2 * t[3]) * ve
        kvo = (ko0 * t[0] + ke0 * t[1] + ko1 * t[2] + ke1 * t[3]) * vo
        ef = _dot(pltpu.bitcast(half_ref[...], BF), kve.astype(BF))
        of = _dot(pltpu.bitcast(half_ref[...], BF), kvo.astype(BF))
        kf = lax.dot_general(pltpu.bitcast(full_ref[...], BF), kk_v[c, :, pl.ds(j * C, C)],
                             (((1,), (1,)), ((), ())), preferred_element_type=F32)

        def store():
            wc, ws = tw_ref[0], tw_ref[1]
            pr = of[:H] * wc + of[H:] * ws
            pi = of[H:] * wc - of[:H] * ws
            for m, (xr, xi) in enumerate(((ef[:H] + pr, ef[H:] + pi), (ef[:H] - pr, ef[H:] - pi))):
                kr, ki = kf[2 * m * H:(2 * m + 1) * H], kf[(2 * m + 1) * H:(2 * m + 2) * H]
                if j == 0:
                    kr = kr + tp[KS:KS + 1, :]
                for n, (xv, kv) in enumerate(((xr, ki - kr), (xi, ki + kr), (xr + xi, kr))):
                    xs[sl][j, pl.ds((3 * m + n) * H, H), :] = xv
                    ks[sl][j, pl.ds((3 * m + n) * H, H), :] = kv
        return store, [(ef, 3), (of, 3), (kf, 12)]

    def conv_mac(sl, ft, sgn, tie):
        def mac(m, j0):
            acc = [[None] * 3 for _ in range(JB)]
            for n in range(3):
                r = pl.ds((3 * m + n) * H + ft * 8, 8)
                for i in range(j0 + JB):
                    xv = tie(xs[sl][i, r, :])
                    for u in range(JB):
                        if j0 + u >= i:
                            p = xv * ks[sl][j0 + u - i, r, :]
                            acc[u][n] = p if acc[u][n] is None else acc[u][n] + p
            return [(a[2] - a[1], a[2] + a[0]) for a in acc]

        z = []
        for m in range(2):
            y = [v for j0 in range(0, NC, JB) for v in mac(m, j0)]
            z.append([y[0]] + [
                (y[j][0] - y[j - 1][1], y[j][1] + y[j - 1][0]) if sgn > 0 else
                (y[j][0] + y[j - 1][1], y[j][1] - y[j - 1][0]) for j in range(1, NC)])
        r = pl.ds(ft * 8, 8)
        wc, ws = tw_ref[0, r, :], tw_ref[1, r, :]
        for j in range(NC):
            (ar, ai), (br, bi) = z[0][j], z[1][j]
            dr, di = ar - br, ai - bi
            for n, val in enumerate((ar + br, ai + bi, dr * wc - di * ws, dr * ws + di * wc)):
                zs[sl][j, pl.ds(n * H + ft * 8, 8), :] = val

    def conv_inv(c, j, sl):
        ye = _dot(pltpu.bitcast(inv_ref[...], BF), zs[sl][j, 0:2 * H, :].astype(BF))
        yo = _dot(pltpu.bitcast(inv_ref[...], BF), zs[sl][j, 2 * H:, :].astype(BF))

        def store():
            y = pltpu.pack_elementwise([ye, yo], packed_dtype=BF)
            y_v[pl.ds(j * C, C), pl.ds(pl.multiple_of(c * W, W), W)] = pltpu.bitcast(y, BF)
        return store, [(ye, 3), (yo, 3)]

    for cp in (*k_copies, *conv_copies(0)):
        cp.wait()
    for c in range(1, AHEAD):
        for cp in conv_copies(c):
            cp.start()

    for j in range(NC):
        conv_fwd(0, j, 0)[0]()

    def conv_step(c, sl, with_fwd, with_inv=True):
        for j in range(NC):
            sts = []
            if with_fwd:
                sts.append(conv_fwd(c + 1, j, 1 - sl))
            if with_inv:
                sts.append(conv_inv(c - 1, j, 1 - sl))
            never = jnp.full((8, W), z_ref[0], jnp.int32) != 0
            outs = [o for st in sts for o in st[1]]
            need = 2 * 2 * 3 * NC
            tot = sum(w for _, w in outs)
            anchors = []
            for val, w in outs:
                cnt = need * w // tot
                nv = val.shape[0] // 8
                anchors += [val[8 * (t * nv // cnt):8 * (t * nv // cnt) + 8] for t in range(cnt)]
            it = iter(anchors)
            tie = lambda xv: jnp.where(never, next(it), xv)
            conv_mac(sl, j, 1, tie)
            conv_mac(sl, j + NC, -1, tie)
            for st in sts:
                st[0]()

    def feed(c):
        for cp in conv_copies(c + 1):
            cp.wait()

        @pl.when(c + AHEAD < NW)
        def _():
            for cp in conv_copies(jnp.minimum(c + AHEAD, NW - 1)):
                cp.start()

        for n, cp in enumerate(w_copies[:3]):
            pl.when(c == NW - AHEAD + n - 1)(cp.start)

    feed(jnp.int32(0))
    conv_step(0, 0, True, False)

    def conv_block(c, carry):
        for u in range(2):
            feed(2 * c + 1 + u)
            conv_step(2 * c + 1 + u, 1 - u, True)
        return carry

    lax.fori_loop(0, 3, conv_block, 0)
    w_copies[3].start()
    conv_step(NW - 1, (NW - 1) % 2, False)

    for j in range(NC):
        conv_inv(NW - 1, j, (NW - 1) % 2)[0]()

    def blk(v, r=0, n=BM):
        return pl.ds(pl.multiple_of((v % NB) * BM + r, 8), n)

    RP = 16
    NP = BM // RP
    never = jnp.full((RP, 128), z_ref[0], jnp.int32) != 0

    def ln_g(x):
        m = yield jnp.mean(x, axis=-1, keepdims=True)
        d = x - m
        v = yield jnp.mean(d * d, axis=-1, keepdims=True)
        r = yield lax.rsqrt(v + EPS)
        return d * r

    def prep(v, src, p):
        rows = blk(v, p * RP, RP)
        x = yield src[rows, :].astype(F32)
        x = x + (yield from ln_g(x)) * y_v[rows, :].astype(F32)
        x_v[rows, :] = x
        xn = yield from ln_g(x)
        xn_v[rows, :] = xn
        la[v % 2, p * RP:(p + 1) * RP, :] = (yield from ln_g(xn)).astype(BF)

    def shift(v, p):
        Q = D // 4
        for g, sh in enumerate((-1, 1, -2, 2)):
            win = yield h_v[blk(v, p * RP, RP + 2 * HALO), g * Q:(g + 1) * Q]
            gb[v % 2, p * RP:(p + 1) * RP, g * Q:(g + 1) * Q] = (
                win[HALO + sh:HALO + sh + RP, :].astype(BF))

    def ln1(v, p):
        x = yield xn_v[blk(v, p * RP, RP), :]
        lb[v % 2, p * RP:(p + 1) * RP, :] = (yield from ln_g(x)).astype(BF)

    def pin(val, anchor):
        if val.shape[1] == 1:
            return jnp.where(never[:, :1], anchor[:, :1], val)
        head = jnp.where(never, anchor, val[:RP, :128])
        if val.shape[0] > RP:
            head = jnp.concatenate([head, val[RP:, :128]], axis=0)
        return jnp.concatenate([head, val[:, 128:]], axis=1)

    class Fill:
        def __init__(self, n_anchor, gap, *stages):
            self.t, self.gap, self.q = 0, gap, {}
            for k, (fn, args, ny) in enumerate(stages):
                period = (n_anchor - gap * ny) // NP
                for p in range(NP):
                    t0 = p * period + (k * period) // len(stages)
                    self.q.setdefault(t0, []).append((fn(*args, p), None))

        def step(self, anchor):
            for gen, val in self.q.pop(self.t, []):
                try:
                    if val is None:
                        val = next(gen)
                    nxt = gen.send(val if anchor is None else pin(val, anchor))
                    self.q.setdefault(self.t + self.gap, []).append((gen, nxt))
                except StopIteration:
                    pass
            self.t += 1

        def feed(self, res):
            for r in range(0, res.shape[0], RP):
                self.step(res[r:r + RP, :])

        def drain(self):
            while self.q:
                self.step(None)

    KC = 512

    def mm(lhs, w_ref, n, fill):
        acc = None
        for k in range(0, lhs.shape[1], KC):
            part = _dot(lhs[:, k:k + KC], w_ref[k:k + KC, n * 128:(n + 1) * 128])
            fill.feed(part)
            acc = part if acc is None else acc + part
        return acc

    NA1 = (D // 128) * (D // KC) * NP
    NA4 = (D // 128) * (F // KC) * NP

    def mix_a(v, *stages):
        if not stages:
            h_v[blk(v, HALO), :] = _gelu(_dot(la[v % 2], w1_v[...]))
            return
        fill = Fill(NA1, 8, *stages)
        lhs = la[v % 2]
        for n in range(D // 128):
            h_v[blk(v, HALO), n * 128:(n + 1) * 128] = _gelu(mm(lhs, w1_v, n, fill))
        fill.drain()

    def mix_b(v):
        xn_v[blk(v), :] = xn_v[blk(v), :] + _dot(gb[v % 2], w2_v[...])

    def mlp(v, *stages):
        rows = blk(v)
        fill = Fill(NA4, GAP, *stages)
        h2 = _gelu(_dot(lb[v % 2], w3_v[...])).astype(BF)
        for n in range(D // 128):
            cols = slice(n * 128, (n + 1) * 128)
            x = mm(h2, w4_v, n, fill) + x_v[rows, cols] + xn_v[rows, cols]
            x_v[rows, cols] = x
            o_v[rows, cols] = x.astype(BF)
        fill.drain()

    def run(*stages):
        Fill(NA4, 1, *stages).drain()

    def out_copy(v):
        return pltpu.make_async_copy(o_v.at[blk(v), :], o_hbm.at[blk(v), :], sem_o.at[v % NB])

    SK = 4
    q_cp, w1_cp, w2_cp, w3_cp, w4_cp = w_copies
    q_cp.wait()
    x_v[(SK + 1) * BM:, :] = q_v[(SK + 1) * BM:, :].astype(F32)
    run((prep, (0, q_v), 10))
    w1_cp.wait()
    w4_cp.start()

    def pro(v, carry):
        mix_a(v, (prep, (v + 1, q_v), 10))
        return carry

    lax.fori_loop(0, SK, pro, 0)
    w2_cp.wait()
    run((shift, (0,), 4), (shift, (1,), 4))
    mix_b(0)
    mix_b(1)
    run((shift, (2,), 4), (ln1, (0,), 4))
    w3_cp.wait()
    w4_cp.wait()

    def main(i, carry):
        mix_b(i + 2)
        mix_a(i + SK)
        mlp(i, (prep, (i + SK + 1, x_v), 10), (shift, (i + 3,), 4), (ln1, (i + 1,), 4))

        @pl.when(i >= NB)
        def _():
            out_copy(i).start()
        return carry

    lax.fori_loop(0, 2 * NB - SK, main, 0)

    def tail(i, carry):
        mix_b(i + 2)
        mlp(i, (shift, (i + 3,), 4), (ln1, (i + 1,), 4))
        out_copy(i).start()
        return carry

    lax.fori_loop(2 * NB - SK, 2 * NB - 2, tail, 0)

    def last(i, carry):
        mlp(i, (ln1, (i + 1,), 4))
        out_copy(i).start()
        return carry

    lax.fori_loop(2 * NB - 2, 2 * NB, last, 0)
    for b in range(NB):
        out_copy(b).wait()


@jax.jit
def pallas_interleave_layers__ssm_conv_h3__mixer_s_mlp__prompt_kernel(
    A_q, A_k, A_v, A_shift_k, A_ssm_k, A_ssm_D, B_x, B_w1, B_w2, B_w3, B_w4,
):
    consts = _dft_mats()
    hbm = pl.BlockSpec(memory_space=pl.ANY)
    vm = pl.BlockSpec(memory_space=pltpu.VMEM)
    out = pl.pallas_call(
        _kernel,
        in_specs=[hbm, hbm, hbm, vm, hbm, vm, hbm, hbm, hbm, hbm, hbm, hbm, hbm, hbm, pl.BlockSpec(memory_space=pltpu.SMEM)],
        out_specs=hbm,
        out_shape=jax.ShapeDtypeStruct((S, D), BF),
        scratch_shapes=[
            *[pltpu.VMEM(a.shape, a.dtype) for a in consts], pltpu.SemaphoreType.DMA((4,)),
            pltpu.VMEM((S, D), BF), pltpu.VMEM((NW, S + KH, W), BF), pltpu.VMEM((NW, S, W), BF),
            pltpu.VMEM((NW, W, S), BF),
            pltpu.VMEM((D, D), BF), pltpu.VMEM((D, D), BF),
            pltpu.VMEM((D, F), BF), pltpu.VMEM((F, D), BF),
            pltpu.VMEM((NW, 8, W), F32),
            *[pltpu.VMEM((NC, 6 * H, W), F32)] * 4, *[pltpu.VMEM((NC, 4 * H, W), F32)] * 2,
            pltpu.VMEM((S, D), BF), pltpu.VMEM((S, D), F32), pltpu.VMEM((S, D), F32),
            pltpu.VMEM((S + 2 * HALO, D), F32), pltpu.VMEM((S, D), BF),
            pltpu.VMEM((2, BM, D), BF), pltpu.VMEM((2, BM, D), BF), pltpu.VMEM((2, BM, D), BF),
            pltpu.SemaphoreType.DMA((3, NW)), pltpu.SemaphoreType.DMA((5,)),
            pltpu.SemaphoreType.DMA((NB,)),
        ],
        compiler_params=pltpu.CompilerParams(vmem_limit_bytes=120 * 1024 * 1024),
    )(A_q.reshape(S, D), A_k.reshape(S, D), A_v.reshape(S, D), A_shift_k.T, A_ssm_k,
      A_ssm_D, B_w1, B_w2, B_w3, B_w4, *consts, np.zeros((1,), np.int32))
    return out.reshape(1, S, D)
```
